```python
import os as _os
_os.environ.setdefault('JAX_PLATFORMS', 'cpu')
import jax
import jax.numpy as jnp

def _softmax(x, axis=-1):
    return jax.nn.softmax(x, axis=axis)

def _gelu(x):
    return jax.nn.gelu(x, approximate=True)

def _silu(x):
    return jax.nn.silu(x)

def _sigmoid(x):
    return jax.nn.sigmoid(x)

def _layernorm(x, axis=-1, eps=1e-05):
    m = jnp.mean(x, axis=axis, keepdims=True)
    v = jnp.var(x, axis=axis, keepdims=True)
    return (x - m) / jnp.sqrt(v + eps)

def _scatter_add(tgt, idx, src, axis=0):
    return tgt.at[idx].add(src)

def _segment_sum(src, seg, n):
    return jax.ops.segment_sum(src, seg, n)

class _Rng:

    def __init__(self, key):
        self._k = key

    def _next(self):
        self._k, sub = jax.random.split(self._k)
        return sub

    def normal(self, shape):
        return jax.random.normal(self._next(), shape, dtype=jnp.bfloat16)

    def randint(self, lo, hi, shape):
        return jax.random.randint(self._next(), shape, lo, hi, dtype=jnp.int32)

    def uniform(self, shape, lo=0.0, hi=1.0):
        return jax.random.uniform(self._next(), shape, jnp.bfloat16, lo, hi)

    def permutation(self, n):
        return jax.random.permutation(self._next(), n)
kernel_name = 'gated_mix__mha_block__memory_aug_recurrent_mem_tr__prompt'

def setup_inputs():
    _rng = _Rng(jax.random.key(int.from_bytes(__import__("os").urandom(4), "little")))
    _w = lambda a: (lambda t: t.astype(jnp.bfloat16) if jnp.issubdtype(t.dtype, jnp.floating) else t)(jnp.asarray(a))

    def _A_setup():
        B, S, D, H = (1, 2048, 512, 32)
        return {'x': _w((lambda *s: _rng.normal(s) * 0.05)(B, S, D)), 'wqkv': _w((lambda *s: _rng.normal(s) * 0.8)(D, 3 * D)), 'wo': _w((lambda *s: _rng.normal(s) * 0.05)(D, D))}
    _A_in = _A_setup()

    def _B_setup():
        B, S, Dm = (1, 2048, 512)
        H, Dh = (32, 128)
        M, seg = (8, 32)
        seg = min(seg, S)
        S = S // seg * seg
        return {'x': _w((lambda *s: _rng.normal(s) * 0.05)(B, S, Dm)), 'mem0': _w((lambda *s: _rng.normal(s) * 0.8)(B, M, Dm)), 'Wq': _w((lambda *s: _rng.normal(s) * 1.6)(Dm, H, Dh) * Dm ** (-0.5)), 'Wk': _w((lambda *s: _rng.normal(s) * 1.6)(Dm, H, Dh) * Dm ** (-0.5)), 'Wv': _w((lambda *s: _rng.normal(s) * 0.8)(Dm, H, Dh) * Dm ** (-0.5)), 'Wo': _w((lambda *s: _rng.normal(s) * 0.8)(H, Dh, Dm) * (H * Dh) ** (-0.5)), 'seg_len': seg}
    _B_in = _B_setup()
    return {'A_x': _A_in['x'], 'A_wqkv': _A_in['wqkv'], 'A_wo': _A_in['wo'], 'B_x': _B_in['x'], 'B_mem0': _B_in['mem0'], 'B_Wq': _B_in['Wq'], 'B_Wk': _B_in['Wk'], 'B_Wv': _B_in['Wv'], 'B_Wo': _B_in['Wo'], 'B_seg_len': _B_in['seg_len'], 'gate_w': _w((lambda *s: _rng.normal(s) * 0.05)(512) * 16.0)}

def reference(A_x, A_wqkv, A_wo, B_x, B_mem0, B_Wq, B_Wk, B_Wv, B_Wo, B_seg_len, gate_w):

    def _A_ref(x, wqkv, wo):
        B, S, D = x.shape
        H = 32
        Dh = D // H
        qkv = (lambda x, *d: x.transpose(*d))((x @ wqkv).reshape(B, S, 3, H, Dh), 2, 0, 3, 1, 4)
        q, k, v = (qkv[0], qkv[1], qkv[2])
        scores = jnp.einsum('bhqd,bhkd->bhqk', q, k) * Dh ** (-0.5)
        p = _softmax(scores, axis=-1)
        o = jnp.einsum('bhqk,bhkd->bhqd', p, v)
        return (lambda x, *d: x.transpose(*d))(o, 0, 2, 1, 3).reshape(B, S, D) @ wo

    def _B_ref(x, mem0, Wq, Wk, Wv, Wo, seg_len):
        B, S, Dm = x.shape
        H, Dh = (Wq.shape[1], Wq.shape[2])
        M = mem0.shape[1]
        scale = Dh ** (-0.5)
        n_seg = S // seg_len
        L = M + seg_len
        idx = jnp.arange(L)
        mask = (idx[:, None] < M) | (idx[:, None] >= idx[None, :])
        mem = mem0
        outs = []
        for s in range(n_seg):
            xs = x[:, s * seg_len:(s + 1) * seg_len, :].copy()
            h = jnp.concatenate([mem, xs], axis=1)
            q = jnp.einsum('btd,dhe->bhte', h, Wq)
            k = jnp.einsum('btd,dhe->bhte', h, Wk)
            v = jnp.einsum('btd,dhe->bhte', h, Wv)
            scores = jnp.einsum('bhqe,bhke->bhqk', q, k) * scale
            scores = jnp.where(mask[None, None], scores, -1000000000.0)
            p = _softmax(scores, axis=-1)
            o = jnp.einsum('bhqk,bhke->bhqe', p, v)
            o = jnp.einsum('bhte,hed->btd', o, Wo)
            mem = o[:, :M, :].copy()
            outs.append(o[:, M:, :])
        return jnp.concatenate(outs, axis=1)
    x = A_x
    g = _sigmoid((x * gate_w).sum(-1, keepdims=True))
    a = _A_ref(x, A_wqkv, A_wo)
    b = _B_ref(x, B_mem0, B_Wq, B_Wk, B_Wv, B_Wo, B_seg_len)
    return g * a + (1 - g) * b
```

```python
import functools
import math

import jax
import jax.numpy as jnp
import jax.experimental.pallas as pl
import jax.experimental.pallas.tpu as pltpu

f32, bf16, u32 = jnp.float32, jnp.bfloat16, jnp.uint32

S, D = 2048, 512
HA, DHA = 32, 16
TQ = 128
GH = 128 // DHA
NG = HA // GH
CH = 32
CHK = 128
LOG2E = math.log2(math.e)
HB, DHB, MEM = 32, 128, 8


def _pack(x):
    return pltpu.bitcast(x, u32)


def _unpack(x):
    return pltpu.bitcast(x, bf16)


def _repack_head_weights(w_ref, tmp, wp_out):
    tmp[...] = _pack(w_ref[...].reshape(D * HB, DHB))
    lo = jnp.uint32(0xFFFF)
    hi = jnp.uint32(0xFFFF0000)
    for hp in range(HB // 2):
        a = tmp[pl.ds(hp, D // 2, stride=HB), :]
        b = tmp[pl.ds(HB // 2 + hp, D // 2, stride=HB), :]
        wp_out[:, (2 * hp) * DHB:(2 * hp + 1) * DHB] = (a & lo) | (b << 16)
        wp_out[:, (2 * hp + 1) * DHB:(2 * hp + 2) * DHB] = (a >> 16) | (b & hi)


def _kernel(x_ref, wqkv_ref, woa_ref, mem0_ref, wq_ref, wk_ref, wv_ref, wob_ref, gw_ref,
            o_ref,
            q_s, kp, vta, st0, st1, pt0, pt1, m0, m1, ot_s, a_s,
            tmp, wq_p, wk_p, wv_p, wo_p, mem_s, *, seg):
    x = x_ref[...]
    q = jnp.dot(x, wqkv_ref[:, 0:D], preferred_element_type=f32)
    q_s[...] = (q * (DHA ** -0.5 * LOG2E)).astype(bf16)
    kp[...] = _pack(jnp.dot(x, wqkv_ref[:, D:2 * D], preferred_element_type=f32).astype(bf16))
    v = jnp.dot(x, wqkv_ref[:, 2 * D:3 * D], preferred_element_type=f32)
    vt = v.T
    rowi = jax.lax.broadcasted_iota(jnp.int32, (16, S), 0)
    ones_blk = jnp.where(rowi == 0, 1.0, 0.0).astype(bf16)
    for h in range(HA):
        vta[pl.ds(h * 16, 8), :] = _pack(vt[h * DHA:(h + 1) * DHA, :].astype(bf16))
        vta[pl.ds(h * 16 + 8, 8), :] = _pack(ones_blk)

    lane_head = jax.lax.broadcasted_iota(jnp.int32, (TQ, 128), 1) // DHA
    NC = S // CHK

    def idx(i):
        g = i % NG
        qb = i // NG
        return g, pl.multiple_of(g * 128, 128), pl.multiple_of(qb * TQ, TQ)

    def build_qm(i):
        g, g0, q0 = idx(i)
        qblk = q_s[pl.ds(q0, TQ), pl.ds(g0, 128)]
        return jnp.concatenate(
            [jnp.where(lane_head == h, qblk, jnp.zeros_like(qblk)) for h in range(GH)], axis=0)

    def scores_chunk(i, qm, st, c, macc):
        g, g0, q0 = idx(i)
        kg = _unpack(kp[c * CHK // 2:(c + 1) * CHK // 2, pl.ds(g0, 128)])
        s = jax.lax.dot_general(kg, qm, (((1,), (1,)), ((), ())), preferred_element_type=f32)
        st[c * CHK:(c + 1) * CHK, :] = s
        cm = jnp.max(s.reshape(CHK // 8, 8, GH * TQ), axis=0)
        return cm if macc is None else jnp.maximum(macc, cm)

    def finish_max(macc, mm):
        mm[...] = jnp.broadcast_to(jnp.max(macc, axis=0, keepdims=True), (8, GH * TQ))

    def softmax_chunk(st, mb, pt, c):
        for cc in range(c * CHK // CH, (c + 1) * CHK // CH):
            p = jnp.exp2(st[cc * CH:(cc + 1) * CH, :] - mb)
            pt[cc * CH // 2:(cc + 1) * CH // 2, :] = _pack(p.astype(bf16))

    def pv_chunk(i, pt, c, R):
        g, g0, q0 = idx(i)
        out = []
        for h in range(GH):
            r0 = pl.multiple_of((g * GH + h) * 16, 16)
            lhs = _unpack(vta[pl.ds(r0, 16), c * CHK:(c + 1) * CHK])
            r = jnp.dot(lhs, _unpack(pt[c * CHK // 2:(c + 1) * CHK // 2, h * TQ:(h + 1) * TQ]),
                        preferred_element_type=f32)
            out.append(r if R is None else R[h] + r)
        return out

    def unit(i_next, st_n, m_n, i, st, mm, pt):
        qm = build_qm(i_next)
        mb = jnp.concatenate([mm[...]] * (CH // 8), axis=0)
        macc = None
        R = None
        for c in range(NC):
            macc = scores_chunk(i_next, qm, st_n, c, macc)
            softmax_chunk(st, mb, pt, c)
            R = pv_chunk(i, pt, c, R)
        finish_max(macc, m_n)
        g, g0, q0 = idx(i)
        for h in range(GH):
            ot_s[pl.ds(pl.multiple_of(g0 + h * DHA, DHA), DHA), pl.ds(q0, TQ)] = (
                R[h][0:DHA] / R[h][DHA:DHA + 1])

    NU = NG * (S // TQ)
    qm0 = build_qm(0)
    macc = None
    for c in range(NC):
        macc = scores_chunk(0, qm0, st0, c, macc)
    finish_max(macc, m0)

    def a_body(j, carry):
        i = 2 * j
        unit(i + 1, st1, m1, i, st0, m0, pt0)
        unit(jnp.minimum(i + 2, NU - 1), st0, m0, i + 1, st1, m1, pt1)
        return carry

    jax.lax.fori_loop(0, NU // 2, a_body, 0)
    a_s[...] = jnp.dot(ot_s[...].T.astype(bf16), woa_ref[...], preferred_element_type=f32)

    _repack_head_weights(wq_ref, tmp, wq_p)
    _repack_head_weights(wk_ref, tmp, wk_p)
    _repack_head_weights(wv_ref, tmp, wv_p)
    wo_p[...] = _pack(wob_ref[...])
    mem_s[...] = mem0_ref[...].astype(f32)
    gw = gw_ref[...].astype(f32)

    L = MEM + seg
    nseg = S // seg
    scale = DHB ** -0.5
    row = jax.lax.broadcasted_iota(jnp.int32, (L, L), 0)
    col = jax.lax.broadcasted_iota(jnp.int32, (L, L), 1)
    mask = (row >= seg) | (col >= seg) | (col <= row)

    def b_body(s, carry):
        x0 = pl.multiple_of(s * seg, seg)
        xs = x_ref[pl.ds(x0, seg), :]
        h = jnp.concatenate([xs, mem_s[...].astype(bf16)], axis=0)
        q = jnp.dot(h, _unpack(wq_p[...]), preferred_element_type=f32).astype(bf16)
        k = jnp.dot(h, _unpack(wk_p[...]), preferred_element_type=f32).astype(bf16)
        v = jnp.dot(h, _unpack(wv_p[...]), preferred_element_type=f32).astype(bf16)
        outs = []
        for hd in range(HB):
            sl = slice(hd * DHB, (hd + 1) * DHB)
            sc = jax.lax.dot_general(q[:, sl], k[:, sl], (((1,), (1,)), ((), ())),
                                     preferred_element_type=f32) * scale
            sc = jnp.where(mask, sc, -1e9)
            mx = jnp.max(sc, axis=-1, keepdims=True)
            p = jnp.exp(sc - mx)
            l = jnp.sum(p, axis=-1, keepdims=True)
            p = (p / l).astype(bf16)
            outs.append(jnp.dot(p, v[:, sl], preferred_element_type=f32).astype(bf16))
        o = jnp.concatenate(outs, axis=1)
        out = jnp.dot(o, _unpack(wo_p[...]), preferred_element_type=f32)
        mem_s[...] = out[seg:].astype(bf16).astype(f32)
        gate = jax.nn.sigmoid(jnp.sum(xs.astype(f32) * gw, axis=-1, keepdims=True))
        o_ref[pl.ds(x0, seg), :] = (gate * a_s[pl.ds(x0, seg), :]
                                    + (1.0 - gate) * out[:seg]).astype(o_ref.dtype)
        return carry

    jax.lax.fori_loop(0, nseg, b_body, 0)


@functools.partial(jax.jit, static_argnames=("B_seg_len",))
def pallas_gated_mix__mha_block__memory_aug_recurrent_mem_tr__prompt_kernel(
    A_x: jax.Array,
    A_wqkv: jax.Array,
    A_wo: jax.Array,
    B_x: jax.Array,
    B_mem0: jax.Array,
    B_Wq: jax.Array,
    B_Wk: jax.Array,
    B_Wv: jax.Array,
    B_Wo: jax.Array,
    B_seg_len: int,
    gate_w: jax.Array,
):
    del B_x
    seg = int(B_seg_len)
    assert A_x.shape == (1, S, D) and B_Wq.shape == (D, HB, DHB) and B_mem0.shape == (1, MEM, D)
    assert S % seg == 0 and seg % 16 == 0

    scratch = [
        pltpu.VMEM((S, D), bf16),
        pltpu.VMEM((S // 2, D), u32),
        pltpu.VMEM((HA * 16, S), u32),
        pltpu.VMEM((S, GH * TQ), f32),
        pltpu.VMEM((S, GH * TQ), f32),
        pltpu.VMEM((S // 2, GH * TQ), u32),
        pltpu.VMEM((S // 2, GH * TQ), u32),
        pltpu.VMEM((8, GH * TQ), f32),
        pltpu.VMEM((8, GH * TQ), f32),
        pltpu.VMEM((D, S), f32),
        pltpu.VMEM((S, D), f32),
        pltpu.VMEM((D * HB // 2, DHB), u32),
        pltpu.VMEM((D // 2, HB * DHB), u32),
        pltpu.VMEM((D // 2, HB * DHB), u32),
        pltpu.VMEM((D // 2, HB * DHB), u32),
        pltpu.VMEM((HB * DHB // 2, D), u32),
        pltpu.VMEM((MEM, D), f32),
    ]
    out = pl.pallas_call(
        functools.partial(_kernel, seg=seg),
        out_shape=jax.ShapeDtypeStruct((S, D), A_x.dtype),
        scratch_shapes=scratch,
        compiler_params=pltpu.CompilerParams(vmem_limit_bytes=120 * 1024 * 1024),
        name="gated_mix_mha_rmt",
    )(
        A_x.reshape(S, D),
        A_wqkv,
        A_wo,
        B_mem0.reshape(MEM, D),
        B_Wq,
        B_Wk,
        B_Wv,
        B_Wo.reshape(HB * DHB, D),
        gate_w.reshape(1, D),
    )
    return out.reshape(1, S, D)
```

```python
import functools
import math

import jax
import jax.numpy as jnp
import jax.experimental.pallas as pl
import jax.experimental.pallas.tpu as pltpu

f32, bf16, u32 = jnp.float32, jnp.bfloat16, jnp.uint32

S, D = 2048, 512
HA, DHA = 32, 16
TQ = 128
GH = 128 // DHA
NG = HA // GH
CH = 32
CHK = 128
LOG2E = math.log2(math.e)
HB, DHB, MEM = 32, 128, 8
NGB = 2
HGB = HB // NGB


def _pack(x):
    return pltpu.bitcast(x, u32)


def _unpack(x):
    return pltpu.bitcast(x, bf16)


def _repack_head_weights(w_ref, tmp, wp_out):
    tmp[...] = _pack(w_ref[...].reshape(D * HB, DHB))
    lo = jnp.uint32(0xFFFF)
    hi = jnp.uint32(0xFFFF0000)
    for hp in range(HB // 2):
        a = tmp[pl.ds(hp, D // 2, stride=HB), :]
        b = tmp[pl.ds(HB // 2 + hp, D // 2, stride=HB), :]
        wp_out[:, (2 * hp) * DHB:(2 * hp + 1) * DHB] = (a & lo) | (b << 16)
        wp_out[:, (2 * hp + 1) * DHB:(2 * hp + 2) * DHB] = (a >> 16) | (b & hi)


def _kernel(x_ref, wqkv_ref, woa_ref, mem0_ref, wq_ref, wk_ref, wv_ref, wob_ref, gw_ref,
            o_ref,
            q_s, kp, vta, st0, st1, pt0, pt1, m0, m1, ot_s, a_s,
            tmp, wq_p, wk_p, wv_p, wo_p, mem_s, *, seg):
    x = x_ref[...]
    q = jnp.dot(x, wqkv_ref[:, 0:D], preferred_element_type=f32)
    q_s[...] = (q * (DHA ** -0.5 * LOG2E)).astype(bf16)
    kp[...] = _pack(jnp.dot(x, wqkv_ref[:, D:2 * D], preferred_element_type=f32).astype(bf16))
    v = jnp.dot(x, wqkv_ref[:, 2 * D:3 * D], preferred_element_type=f32)
    vt = v.T
    rowi = jax.lax.broadcasted_iota(jnp.int32, (16, S), 0)
    ones_blk = jnp.where(rowi == 0, 1.0, 0.0).astype(bf16)
    for h in range(HA):
        vta[pl.ds(h * 16, 8), :] = _pack(vt[h * DHA:(h + 1) * DHA, :].astype(bf16))
        vta[pl.ds(h * 16 + 8, 8), :] = _pack(ones_blk)

    lane_head = jax.lax.broadcasted_iota(jnp.int32, (TQ, 128), 1) // DHA
    NC = S // CHK

    def idx(i):
        g = i % NG
        qb = i // NG
        return g, pl.multiple_of(g * 128, 128), pl.multiple_of(qb * TQ, TQ)

    def build_qm(i):
        g, g0, q0 = idx(i)
        qblk = q_s[pl.ds(q0, TQ), pl.ds(g0, 128)]
        return jnp.concatenate(
            [jnp.where(lane_head == h, qblk, jnp.zeros_like(qblk)) for h in range(GH)], axis=0)

    def scores_chunk(i, qm, st, c, macc):
        g, g0, q0 = idx(i)
        kg = _unpack(kp[c * CHK // 2:(c + 1) * CHK // 2, pl.ds(g0, 128)])
        s = jax.lax.dot_general(kg, qm, (((1,), (1,)), ((), ())), preferred_element_type=f32)
        st[c * CHK:(c + 1) * CHK, :] = s
        cm = jnp.max(s.reshape(CHK // 8, 8, GH * TQ), axis=0)
        return cm if macc is None else jnp.maximum(macc, cm)

    def finish_max(macc, mm):
        mm[...] = jnp.broadcast_to(jnp.max(macc, axis=0, keepdims=True), (8, GH * TQ))

    def softmax_chunk(st, mb, pt, c):
        for cc in range(c * CHK // CH, (c + 1) * CHK // CH):
            p = jnp.exp2(st[cc * CH:(cc + 1) * CH, :] - mb)
            pt[cc * CH // 2:(cc + 1) * CH // 2, :] = _pack(p.astype(bf16))

    def pv_chunk(i, pt, c, R):
        g, g0, q0 = idx(i)
        out = []
        for h in range(GH):
            r0 = pl.multiple_of((g * GH + h) * 16, 16)
            lhs = _unpack(vta[pl.ds(r0, 16), c * CHK:(c + 1) * CHK])
            r = jnp.dot(lhs, _unpack(pt[c * CHK // 2:(c + 1) * CHK // 2, h * TQ:(h + 1) * TQ]),
                        preferred_element_type=f32)
            out.append(r if R is None else R[h] + r)
        return out

    def unit(i_next, st_n, m_n, i, st, mm, pt):
        qm = build_qm(i_next)
        mb = jnp.concatenate([mm[...]] * (CH // 8), axis=0)
        macc = None
        R = None
        for c in range(NC):
            macc = scores_chunk(i_next, qm, st_n, c, macc)
            softmax_chunk(st, mb, pt, c)
            R = pv_chunk(i, pt, c, R)
        finish_max(macc, m_n)
        g, g0, q0 = idx(i)
        for h in range(GH):
            ot_s[pl.ds(pl.multiple_of(g0 + h * DHA, DHA), DHA), pl.ds(q0, TQ)] = (
                R[h][0:DHA] / R[h][DHA:DHA + 1])

    NU = NG * (S // TQ)
    qm0 = build_qm(0)
    macc = None
    for c in range(NC):
        macc = scores_chunk(0, qm0, st0, c, macc)
    finish_max(macc, m0)

    def a_body(j, carry):
        i = 2 * j
        unit(i + 1, st1, m1, i, st0, m0, pt0)
        unit(jnp.minimum(i + 2, NU - 1), st0, m0, i + 1, st1, m1, pt1)
        return carry

    jax.lax.fori_loop(0, NU // 2, a_body, 0)
    a_s[...] = jnp.dot(ot_s[...].T.astype(bf16), woa_ref[...], preferred_element_type=f32)

    _repack_head_weights(wq_ref, tmp, wq_p)
    _repack_head_weights(wk_ref, tmp, wk_p)
    _repack_head_weights(wv_ref, tmp, wv_p)
    wo_p[...] = _pack(wob_ref[...])
    mem_s[...] = mem0_ref[...].astype(f32)
    gw = gw_ref[...].astype(f32)

    L = MEM + seg
    nseg = S // seg
    scale = DHB ** -0.5
    gw_cols = HGB * DHB
    row = jax.lax.broadcasted_iota(jnp.int32, (L, L), 0)
    col = jax.lax.broadcasted_iota(jnp.int32, (L, L), 1)
    mask = (row >= seg) | (col >= seg) | (col <= row)

    def proj1(hb, w_p, g):
        return jnp.dot(hb, _unpack(w_p[:, g * gw_cols:(g + 1) * gw_cols]), preferred_element_type=f32)

    def scores_b(q, k):
        q = q.astype(bf16)
        k = k.astype(bf16)
        return [jax.lax.dot_general(q[:, hd * DHB:(hd + 1) * DHB], k[:, hd * DHB:(hd + 1) * DHB],
                                    (((1,), (1,)), ((), ())), preferred_element_type=f32)
                for hd in range(HGB)]

    def softmax_b(scs):
        out = []
        for sc in scs:
            sc = jnp.where(mask, sc * scale, -1e9)
            mx = jnp.max(sc, axis=-1, keepdims=True)
            p = jnp.exp(sc - mx)
            l = jnp.sum(p, axis=-1, keepdims=True)
            out.append((p / l).astype(bf16))
        return out

    def pv_b(ps, v):
        v = v.astype(bf16)
        return jnp.concatenate(
            [jnp.dot(ps[hd], v[:, hd * DHB:(hd + 1) * DHB], preferred_element_type=f32)
             for hd in range(HGB)], axis=1)

    def oproj1(lhs, g):
        return jnp.dot(lhs.astype(bf16), _unpack(wo_p[g * gw_cols // 2:(g + 1) * gw_cols // 2, :]),
                       preferred_element_type=f32)

    def step(hrows, tokens, olhs):
        hb = hrows.astype(bf16)
        proj = [None] * NGB
        proj[0] = [proj1(hb, w, 0) for w in (wq_p, wk_p, wv_p)]
        acc = None
        o_g = [None] * NGB
        for g in range(NGB):
            q, k, v = (tokens(g, i, a) for i, a in enumerate(proj[g]))
            scs = scores_b(q, k)
            if g + 1 < NGB:
                nq = proj1(hb, wq_p, g + 1)
            ps = softmax_b(scs)
            o_g[g] = pv_b(ps, v)
            if g + 1 < NGB:
                proj[g + 1] = [nq, proj1(hb, wk_p, g + 1), proj1(hb, wv_p, g + 1)]
            if g >= 1:
                r = oproj1(olhs(g - 1, o_g[g - 1]), g - 1)
                acc = r if acc is None else acc + r
        r = oproj1(olhs(NGB - 1, o_g[NGB - 1]), NGB - 1)
        acc = r if acc is None else acc + r
        return acc, proj

    xtra = MEM

    def b_body(j, carry):
        x0 = pl.multiple_of(j * 2 * seg, 2 * seg)
        xs = x_ref[pl.ds(x0, 2 * seg), :].astype(f32)
        mem = mem_s[...]
        held = {}

        def tokens_e(g, i, a):
            return jnp.concatenate([a[0:seg], a[seg + xtra:seg + xtra + MEM]], axis=0)

        def olhs_e(g, o):
            held[g] = o[seg - xtra:seg]
            return jnp.concatenate([o[seg:L], o[0:seg - xtra]], axis=0)

        oe, proj_e = step(jnp.concatenate([xs[0:seg + xtra], mem], axis=0), tokens_e, olhs_e)
        mem = oe[0:MEM].astype(bf16).astype(f32)

        def tokens_o(g, i, a):
            return jnp.concatenate([proj_e[g][i][seg:seg + xtra], a], axis=0)

        def olhs_o(g, o):
            return jnp.concatenate([o[seg:L], held[g], o[0:seg]], axis=0)

        oo, _ = step(jnp.concatenate([xs[seg + xtra:2 * seg], mem], axis=0), tokens_o, olhs_o)
        mem_s[...] = oo[0:MEM].astype(bf16).astype(f32)
        b = jnp.concatenate([oe[MEM:], oo[MEM:]], axis=0)
        gate = jax.nn.sigmoid(jnp.sum(xs * gw, axis=-1, keepdims=True))
        o_ref[pl.ds(x0, 2 * seg), :] = (gate * a_s[pl.ds(x0, 2 * seg), :]
                                        + (1.0 - gate) * b).astype(o_ref.dtype)
        return carry

    jax.lax.fori_loop(0, nseg // 2, b_body, 0)


@functools.partial(jax.jit, static_argnames=("B_seg_len",))
def pallas_gated_mix__mha_block__memory_aug_recurrent_mem_tr__prompt_kernel(
    A_x: jax.Array,
    A_wqkv: jax.Array,
    A_wo: jax.Array,
    B_x: jax.Array,
    B_mem0: jax.Array,
    B_Wq: jax.Array,
    B_Wk: jax.Array,
    B_Wv: jax.Array,
    B_Wo: jax.Array,
    B_seg_len: int,
    gate_w: jax.Array,
):
    del B_x
    seg = int(B_seg_len)
    assert A_x.shape == (1, S, D) and B_Wq.shape == (D, HB, DHB) and B_mem0.shape == (1, MEM, D)
    assert S % (2 * seg) == 0 and seg % 16 == 0 and seg > MEM

    scratch = [
        pltpu.VMEM((S, D), bf16),
        pltpu.VMEM((S // 2, D), u32),
        pltpu.VMEM((HA * 16, S), u32),
        pltpu.VMEM((S, GH * TQ), f32),
        pltpu.VMEM((S, GH * TQ), f32),
        pltpu.VMEM((S // 2, GH * TQ), u32),
        pltpu.VMEM((S // 2, GH * TQ), u32),
        pltpu.VMEM((8, GH * TQ), f32),
        pltpu.VMEM((8, GH * TQ), f32),
        pltpu.VMEM((D, S), f32),
        pltpu.VMEM((S, D), f32),
        pltpu.VMEM((D * HB // 2, DHB), u32),
        pltpu.VMEM((D // 2, HB * DHB), u32),
        pltpu.VMEM((D // 2, HB * DHB), u32),
        pltpu.VMEM((D // 2, HB * DHB), u32),
        pltpu.VMEM((HB * DHB // 2, D), u32),
        pltpu.VMEM((MEM, D), f32),
    ]
    out = pl.pallas_call(
        functools.partial(_kernel, seg=seg),
        out_shape=jax.ShapeDtypeStruct((S, D), A_x.dtype),
        scratch_shapes=scratch,
        compiler_params=pltpu.CompilerParams(vmem_limit_bytes=120 * 1024 * 1024),
        name="gated_mix_mha_rmt",
    )(
        A_x.reshape(S, D),
        A_wqkv,
        A_wo,
        B_mem0.reshape(MEM, D),
        B_Wq,
        B_Wk,
        B_Wv,
        B_Wo.reshape(HB * DHB, D),
        gate_w.reshape(1, D),
    )
    return out.reshape(1, S, D)
```

```python
import functools
import math

import jax
import jax.numpy as jnp
import jax.experimental.pallas as pl
import jax.experimental.pallas.tpu as pltpu

f32, bf16, u32 = jnp.float32, jnp.bfloat16, jnp.uint32

S, D = 2048, 512
HA, DHA = 32, 16
TQ = 128
GH = 128 // DHA
NG = HA // GH
CH = 32
CHK = 128
LOG2E = math.log2(math.e)
HB, DHB, MEM = 32, 128, 8
NGB = 2
HGB = HB // NGB


def _pack(x):
    return pltpu.bitcast(x, u32)


def _unpack(x):
    return pltpu.bitcast(x, bf16)


def _kernel(x_ref, wqkv_ref, woa_ref, mem0_ref, wq_hbm, wk_hbm, wv_hbm, wob_hbm, gw_ref,
            o_ref,
            q_s, kp, vta, st0, st1, pt0, pt1, m0, m1, ot_s, a_s,
            wq_raw, wk_raw, wv_raw, wo_raw, wq_p, wk_p, wv_p, wo_p, mem_s, sems, *, seg):
    w_copies = [pltpu.make_async_copy(src, dst, sems.at[i]) for i, (src, dst) in enumerate(
        [(wq_hbm, wq_raw), (wk_hbm, wk_raw), (wv_hbm, wv_raw), (wob_hbm, wo_raw)])]
    for cp in w_copies:
        cp.start()

    x = x_ref[...]
    q = jnp.dot(x, wqkv_ref[:, 0:D], preferred_element_type=f32)
    q_s[...] = (q * (DHA ** -0.5 * LOG2E)).astype(bf16)
    kp[...] = _pack(jnp.dot(x, wqkv_ref[:, D:2 * D], preferred_element_type=f32).astype(bf16))
    v = jnp.dot(x, wqkv_ref[:, 2 * D:3 * D], preferred_element_type=f32)
    vt = v.T
    rowi = jax.lax.broadcasted_iota(jnp.int32, (16, S), 0)
    ones_blk = jnp.where(rowi == 0, 1.0, 0.0).astype(bf16)
    for h in range(HA):
        vta[pl.ds(h * 16, 8), :] = _pack(vt[h * DHA:(h + 1) * DHA, :].astype(bf16))
        vta[pl.ds(h * 16 + 8, 8), :] = _pack(ones_blk)

    lane_head = jax.lax.broadcasted_iota(jnp.int32, (TQ, 128), 1) // DHA
    NC = S // CHK

    def idx(i):
        g = i % NG
        qb = i // NG
        return g, pl.multiple_of(g * 128, 128), pl.multiple_of(qb * TQ, TQ)

    def build_qm(i):
        g, g0, q0 = idx(i)
        qblk = q_s[pl.ds(q0, TQ), pl.ds(g0, 128)]
        return jnp.concatenate(
            [jnp.where(lane_head == h, qblk, jnp.zeros_like(qblk)) for h in range(GH)], axis=0)

    def scores_chunk(i, qm, st, c, macc):
        g, g0, q0 = idx(i)
        kg = _unpack(kp[c * CHK // 2:(c + 1) * CHK // 2, pl.ds(g0, 128)])
        s = jax.lax.dot_general(kg, qm, (((1,), (1,)), ((), ())), preferred_element_type=f32)
        st[c * CHK:(c + 1) * CHK, :] = s
        cm = jnp.max(s.reshape(CHK // 8, 8, GH * TQ), axis=0)
        return cm if macc is None else jnp.maximum(macc, cm)

    def finish_max(macc, mm):
        mm[...] = jnp.broadcast_to(jnp.max(macc, axis=0, keepdims=True), (8, GH * TQ))

    def softmax_chunk(st, mb, pt, c):
        for cc in range(c * CHK // CH, (c + 1) * CHK // CH):
            p = jnp.exp2(st[cc * CH:(cc + 1) * CH, :] - mb)
            pt[cc * CH // 2:(cc + 1) * CH // 2, :] = _pack(p.astype(bf16))

    def pv_chunk(i, pt, c, R):
        g, g0, q0 = idx(i)
        out = []
        for h in range(GH):
            r0 = pl.multiple_of((g * GH + h) * 16, 16)
            lhs = _unpack(vta[pl.ds(r0, 16), c * CHK:(c + 1) * CHK])
            r = jnp.dot(lhs, _unpack(pt[c * CHK // 2:(c + 1) * CHK // 2, h * TQ:(h + 1) * TQ]),
                        preferred_element_type=f32)
            out.append(r if R is None else R[h] + r)
        return out

    def unit(i_next, st_n, m_n, i, st, mm, pt):
        qm = build_qm(i_next)
        mb = jnp.concatenate([mm[...]] * (CH // 8), axis=0)
        macc = None
        R = None
        for c in range(NC):
            macc = scores_chunk(i_next, qm, st_n, c, macc)
            softmax_chunk(st, mb, pt, c)
            R = pv_chunk(i, pt, c, R)
        finish_max(macc, m_n)
        g, g0, q0 = idx(i)
        for h in range(GH):
            ot_s[pl.ds(pl.multiple_of(g0 + h * DHA, DHA), DHA), pl.ds(q0, TQ)] = (
                R[h][0:DHA] / R[h][DHA:DHA + 1])

    NU = NG * (S // TQ)
    qm0 = build_qm(0)
    macc = None
    for c in range(NC):
        macc = scores_chunk(0, qm0, st0, c, macc)
    finish_max(macc, m0)

    def a_body(j, carry):
        i = 2 * j
        unit(i + 1, st1, m1, i, st0, m0, pt0)
        unit(jnp.minimum(i + 2, NU - 1), st0, m0, i + 1, st1, m1, pt1)
        return carry

    jax.lax.fori_loop(0, NU // 2, a_body, 0)
    a_s[...] = jnp.dot(ot_s[...].T.astype(bf16), woa_ref[...], preferred_element_type=f32)

    for cp, raw, packed in zip(w_copies[:3], (wq_raw, wk_raw, wv_raw), (wq_p, wk_p, wv_p)):
        cp.wait()
        packed[...] = _pack(raw[...].reshape(D, HB * DHB))
    w_copies[3].wait()
    wo_p[...] = _pack(wo_raw[...])
    mem_s[...] = mem0_ref[...].astype(f32)
    gw = gw_ref[...].astype(f32)

    L = MEM + seg
    nseg = S // seg
    scale = DHB ** -0.5
    gw_cols = HGB * DHB
    row = jax.lax.broadcasted_iota(jnp.int32, (L, L), 0)
    col = jax.lax.broadcasted_iota(jnp.int32, (L, L), 1)
    mask = (row >= seg) | (col >= seg) | (col <= row)

    def proj1(hb, w_p, g):
        return jnp.dot(hb, _unpack(w_p[:, g * gw_cols:(g + 1) * gw_cols]), preferred_element_type=f32)

    def scores_b(q, k):
        q = q.astype(bf16)
        k = k.astype(bf16)
        return [jax.lax.dot_general(q[:, hd * DHB:(hd + 1) * DHB], k[:, hd * DHB:(hd + 1) * DHB],
                                    (((1,), (1,)), ((), ())), preferred_element_type=f32)
                for hd in range(HGB)]

    def softmax_b(scs):
        out = []
        for sc in scs:
            sc = jnp.where(mask, sc * scale, -1e9)
            mx = jnp.max(sc, axis=-1, keepdims=True)
            p = jnp.exp(sc - mx)
            l = jnp.sum(p, axis=-1, keepdims=True)
            out.append((p / l).astype(bf16))
        return out

    def pv_b(ps, v):
        v = v.astype(bf16)
        return jnp.concatenate(
            [jnp.dot(ps[hd], v[:, hd * DHB:(hd + 1) * DHB], preferred_element_type=f32)
             for hd in range(HGB)], axis=1)

    def oproj1(lhs, g):
        return jnp.dot(lhs.astype(bf16), _unpack(wo_p[g * gw_cols // 2:(g + 1) * gw_cols // 2, :]),
                       preferred_element_type=f32)

    def step(hrows, tokens, olhs):
        hb = hrows.astype(bf16)
        proj = [None] * NGB
        proj[0] = [proj1(hb, w, 0) for w in (wq_p, wk_p, wv_p)]
        acc = None
        o_g = [None] * NGB
        for g in range(NGB):
            q, k, v = (tokens(g, i, a) for i, a in enumerate(proj[g]))
            scs = scores_b(q, k)
            if g + 1 < NGB:
                nq = proj1(hb, wq_p, g + 1)
            ps = softmax_b(scs)
            o_g[g] = pv_b(ps, v)
            if g + 1 < NGB:
                proj[g + 1] = [nq, proj1(hb, wk_p, g + 1), proj1(hb, wv_p, g + 1)]
            if g >= 1:
                r = oproj1(olhs(g - 1, o_g[g - 1]), g - 1)
                acc = r if acc is None else acc + r
        r = oproj1(olhs(NGB - 1, o_g[NGB - 1]), NGB - 1)
        acc = r if acc is None else acc + r
        return acc, proj

    xtra = MEM

    def b_body(j, carry):
        x0 = pl.multiple_of(j * 2 * seg, 2 * seg)
        xs = x_ref[pl.ds(x0, 2 * seg), :].astype(f32)
        mem = mem_s[...]
        held = {}

        def tokens_e(g, i, a):
            return jnp.concatenate([a[0:seg], a[seg + xtra:seg + xtra + MEM]], axis=0)

        def olhs_e(g, o):
            held[g] = o[seg - xtra:seg]
            return jnp.concatenate([o[seg:L], o[0:seg - xtra]], axis=0)

        oe, proj_e = step(jnp.concatenate([xs[0:seg + xtra], mem], axis=0), tokens_e, olhs_e)
        mem = oe[0:MEM].astype(bf16).astype(f32)

        def tokens_o(g, i, a):
            return jnp.concatenate([proj_e[g][i][seg:seg + xtra], a], axis=0)

        def olhs_o(g, o):
            return jnp.concatenate([o[seg:L], held[g], o[0:seg]], axis=0)

        oo, _ = step(jnp.concatenate([xs[seg + xtra:2 * seg], mem], axis=0), tokens_o, olhs_o)
        mem_s[...] = oo[0:MEM].astype(bf16).astype(f32)
        b = jnp.concatenate([oe[MEM:], oo[MEM:]], axis=0)
        gate = jax.nn.sigmoid(jnp.sum(xs * gw, axis=-1, keepdims=True))
        o_ref[pl.ds(x0, 2 * seg), :] = (gate * a_s[pl.ds(x0, 2 * seg), :]
                                        + (1.0 - gate) * b).astype(o_ref.dtype)
        return carry

    jax.lax.fori_loop(0, nseg // 2, b_body, 0)


@functools.partial(jax.jit, static_argnames=("B_seg_len",))
def pallas_gated_mix__mha_block__memory_aug_recurrent_mem_tr__prompt_kernel(
    A_x: jax.Array,
    A_wqkv: jax.Array,
    A_wo: jax.Array,
    B_x: jax.Array,
    B_mem0: jax.Array,
    B_Wq: jax.Array,
    B_Wk: jax.Array,
    B_Wv: jax.Array,
    B_Wo: jax.Array,
    B_seg_len: int,
    gate_w: jax.Array,
):
    del B_x
    seg = int(B_seg_len)
    assert A_x.shape == (1, S, D) and B_Wq.shape == (D, HB, DHB) and B_mem0.shape == (1, MEM, D)
    assert S % (2 * seg) == 0 and seg % 16 == 0 and seg > MEM

    scratch = [
        pltpu.VMEM((S, D), bf16),
        pltpu.VMEM((S // 2, D), u32),
        pltpu.VMEM((HA * 16, S), u32),
        pltpu.VMEM((S, GH * TQ), f32),
        pltpu.VMEM((S, GH * TQ), f32),
        pltpu.VMEM((S // 2, GH * TQ), u32),
        pltpu.VMEM((S // 2, GH * TQ), u32),
        pltpu.VMEM((8, GH * TQ), f32),
        pltpu.VMEM((8, GH * TQ), f32),
        pltpu.VMEM((D, S), f32),
        pltpu.VMEM((S, D), f32),
        pltpu.VMEM((D, HB, DHB), bf16),
        pltpu.VMEM((D, HB, DHB), bf16),
        pltpu.VMEM((D, HB, DHB), bf16),
        pltpu.VMEM((HB * DHB, D), bf16),
        pltpu.VMEM((D // 2, HB * DHB), u32),
        pltpu.VMEM((D // 2, HB * DHB), u32),
        pltpu.VMEM((D // 2, HB * DHB), u32),
        pltpu.VMEM((HB * DHB // 2, D), u32),
        pltpu.VMEM((MEM, D), f32),
        pltpu.SemaphoreType.DMA((4,)),
    ]
    vmem_full = pl.BlockSpec(memory_space=pltpu.VMEM)
    hbm_full = pl.BlockSpec(memory_space=pl.ANY)
    out = pl.pallas_call(
        functools.partial(_kernel, seg=seg),
        out_shape=jax.ShapeDtypeStruct((S, D), A_x.dtype),
        in_specs=[vmem_full] * 4 + [hbm_full] * 4 + [vmem_full],
        out_specs=vmem_full,
        scratch_shapes=scratch,
        compiler_params=pltpu.CompilerParams(vmem_limit_bytes=120 * 1024 * 1024),
        name="gated_mix_mha_rmt",
    )(
        A_x.reshape(S, D),
        A_wqkv,
        A_wo,
        B_mem0.reshape(MEM, D),
        B_Wq,
        B_Wk,
        B_Wv,
        B_Wo.reshape(HB * DHB, D),
        gate_w.reshape(1, D),
    )
    return out.reshape(1, S, D)
```

```python
import functools
import math

import jax
import jax.numpy as jnp
import jax.experimental.pallas as pl
import jax.experimental.pallas.tpu as pltpu

f32, bf16, u32 = jnp.float32, jnp.bfloat16, jnp.uint32

S, D = 2048, 512
HA, DHA = 32, 16
TQ = 128
GH = 128 // DHA
NG = HA // GH
CH = 32
CHK = 128
SKEW = (S // CHK) // 2
LOG2E = math.log2(math.e)
HB, DHB, MEM = 32, 128, 8
BND = (0, 10, 22, 32)
NGB = len(BND) - 1


def _pack(x):
    return pltpu.bitcast(x, u32)


def _unpack(x):
    return pltpu.bitcast(x, bf16)


def _kernel(x_ref, wqkv_ref, woa_ref, mem0_ref, wq_hbm, wk_hbm, wv_hbm, wob_hbm, gw_ref,
            o_ref,
            q_s, kp, vta, st0, st1, pt0, pt1, m0, m1, mc, ot_s, a_s,
            wq_raw, wk_raw, wv_raw, wo_raw, wq_p, wk_p, wv_p, wo_p, mem_s, sems, *, seg):
    w_copies = [pltpu.make_async_copy(src, dst, sems.at[i]) for i, (src, dst) in enumerate(
        [(wq_hbm, wq_raw), (wk_hbm, wk_raw), (wv_hbm, wv_raw), (wob_hbm, wo_raw)])]
    for cp in w_copies:
        cp.start()

    x = x_ref[...]
    q = jnp.dot(x, wqkv_ref[:, 0:D], preferred_element_type=f32)
    q_s[...] = (q * (DHA ** -0.5 * LOG2E)).astype(bf16)
    kp[...] = _pack(jnp.dot(x, wqkv_ref[:, D:2 * D], preferred_element_type=f32).astype(bf16))
    v = jnp.dot(x, wqkv_ref[:, 2 * D:3 * D], preferred_element_type=f32)
    vt = v.T
    rowi = jax.lax.broadcasted_iota(jnp.int32, (16, S), 0)
    ones_blk = jnp.where(rowi == 0, 1.0, 0.0).astype(bf16)
    for h in range(HA):
        vta[pl.ds(h * 16, 8), :] = _pack(vt[h * DHA:(h + 1) * DHA, :].astype(bf16))
        vta[pl.ds(h * 16 + 8, 8), :] = _pack(ones_blk)

    lane_head = jax.lax.broadcasted_iota(jnp.int32, (TQ, 128), 1) // DHA
    NC = S // CHK

    def idx(i):
        g = i % NG
        qb = i // NG
        return g, pl.multiple_of(g * 128, 128), pl.multiple_of(qb * TQ, TQ)

    def build_qm(i):
        g, g0, q0 = idx(i)
        qblk = q_s[pl.ds(q0, TQ), pl.ds(g0, 128)]
        return jnp.concatenate(
            [jnp.where(lane_head == h, qblk, jnp.zeros_like(qblk)) for h in range(GH)], axis=0)

    def scores_chunk(i, qm, st, c, macc):
        g, g0, q0 = idx(i)
        kg = _unpack(kp[c * CHK // 2:(c + 1) * CHK // 2, pl.ds(g0, 128)])
        s = jax.lax.dot_general(kg, qm, (((1,), (1,)), ((), ())), preferred_element_type=f32)
        st[c * CHK:(c + 1) * CHK, :] = s
        cm = jnp.max(s.reshape(CHK // 8, 8, GH * TQ), axis=0)
        return cm if macc is None else jnp.maximum(macc, cm)

    def finish_max(macc, mm):
        mm[...] = jnp.broadcast_to(jnp.max(macc, axis=0, keepdims=True), (8, GH * TQ))

    def softmax_chunk(st, mb, pt, c):
        for cc in range(c * CHK // CH, (c + 1) * CHK // CH):
            p = jnp.exp2(st[cc * CH:(cc + 1) * CH, :] - mb)
            pt[cc * CH // 2:(cc + 1) * CH // 2, :] = _pack(p.astype(bf16))

    def pv_chunk(i, pt, c, R):
        g, g0, q0 = idx(i)
        out = []
        for h in range(GH):
            r0 = pl.multiple_of((g * GH + h) * 16, 16)
            lhs = _unpack(vta[pl.ds(r0, 16), c * CHK:(c + 1) * CHK])
            r = jnp.dot(lhs, _unpack(pt[c * CHK // 2:(c + 1) * CHK // 2, h * TQ:(h + 1) * TQ]),
                        preferred_element_type=f32)
            out.append(r if R is None else R[h] + r)
        return out

    def unit(i, st_cur, m_cur, pt, st_oth, m_oth, macc):
        u1 = jnp.minimum(i + 1, NU - 1)
        u2 = jnp.minimum(i + 2, NU - 1)
        qm1 = build_qm(u1)
        qm2 = None
        mb = jnp.concatenate([m_cur[...]] * (CH // 8), axis=0)
        R = None
        for c in range(NC):
            cs = c + SKEW
            if cs < NC:
                macc = scores_chunk(u1, qm1, st_oth, cs, macc)
            else:
                if cs == NC:
                    finish_max(macc, m_oth)
                    macc = None
                    qm2 = build_qm(u2)
                macc = scores_chunk(u2, qm2, st_cur, cs - NC, macc)
            softmax_chunk(st_cur, mb, pt, c)
            R = pv_chunk(i, pt, c, R)
        g, g0, q0 = idx(i)
        for h in range(GH):
            ot_s[pl.ds(pl.multiple_of(g0 + h * DHA, DHA), DHA), pl.ds(q0, TQ)] = (
                R[h][0:DHA] / R[h][DHA:DHA + 1])
        return macc

    NU = NG * (S // TQ)
    qm0 = build_qm(0)
    macc = None
    for c in range(NC):
        macc = scores_chunk(0, qm0, st0, c, macc)
    finish_max(macc, m0)
    qm1 = build_qm(1)
    macc = None
    for c in range(SKEW):
        macc = scores_chunk(1, qm1, st1, c, macc)
    mc[...] = macc

    def a_body(j, carry):
        i = 2 * j
        macc = unit(i, st0, m0, pt0, st1, m1, mc[...])
        mc[...] = unit(i + 1, st1, m1, pt1, st0, m0, macc)
        return carry

    jax.lax.fori_loop(0, NU // 2, a_body, 0)
    a_s[...] = jnp.dot(ot_s[...].T.astype(bf16), woa_ref[...], preferred_element_type=f32)

    for cp, raw, packed in zip(w_copies[:3], (wq_raw, wk_raw, wv_raw), (wq_p, wk_p, wv_p)):
        cp.wait()
        packed[...] = _pack(raw[...].reshape(D, HB * DHB))
    w_copies[3].wait()
    wo_p[...] = _pack(wo_raw[...])
    mem_s[...] = mem0_ref[...].astype(f32)
    gw = gw_ref[...].astype(f32)

    L = MEM + seg
    nseg = S // seg
    scale = DHB ** -0.5
    row = jax.lax.broadcasted_iota(jnp.int32, (L, L), 0)
    col = jax.lax.broadcasted_iota(jnp.int32, (L, L), 1)
    mask = (row >= seg) | (col >= seg) | (col <= row)

    def proj1(hb, w_p, g):
        return jnp.dot(hb, _unpack(w_p[:, BND[g] * DHB:BND[g + 1] * DHB]), preferred_element_type=f32)

    def scores_b(q, k):
        q = q.astype(bf16)
        k = k.astype(bf16)
        return [jax.lax.dot_general(q[:, hd * DHB:(hd + 1) * DHB], k[:, hd * DHB:(hd + 1) * DHB],
                                    (((1,), (1,)), ((), ())), preferred_element_type=f32)
                for hd in range(q.shape[1] // DHB)]

    def softmax_b(scs):
        out = []
        for sc in scs:
            sc = jnp.where(mask, sc * scale, -1e9)
            mx = jnp.max(sc, axis=-1, keepdims=True)
            p = jnp.exp(sc - mx)
            l = jnp.sum(p, axis=-1, keepdims=True)
            out.append((p / l).astype(bf16))
        return out

    def pv_b(ps, v):
        v = v.astype(bf16)
        return jnp.concatenate(
            [jnp.dot(ps[hd], v[:, hd * DHB:(hd + 1) * DHB], preferred_element_type=f32)
             for hd in range(len(ps))], axis=1)

    def oproj1(lhs, g):
        return jnp.dot(lhs.astype(bf16), _unpack(wo_p[BND[g] * DHB // 2:BND[g + 1] * DHB // 2, :]),
                       preferred_element_type=f32)

    def step(hrows, tokens, olhs):
        hb = hrows.astype(bf16)
        proj = [None] * NGB
        proj[0] = [proj1(hb, w, 0) for w in (wq_p, wk_p, wv_p)]
        acc = None
        o_g = [None] * NGB
        for g in range(NGB):
            q, k, v = (tokens(g, i, a) for i, a in enumerate(proj[g]))
            scs = scores_b(q, k)
            if g + 1 < NGB:
                nq = proj1(hb, wq_p, g + 1)
            if g >= 1:
                r = oproj1(olhs(g - 1, o_g[g - 1]), g - 1)
                acc = r if acc is None else acc + r
            ps = softmax_b(scs)
            o_g[g] = pv_b(ps, v)
            if g + 1 < NGB:
                proj[g + 1] = [nq, proj1(hb, wk_p, g + 1), proj1(hb, wv_p, g + 1)]
        r = oproj1(olhs(NGB - 1, o_g[NGB - 1]), NGB - 1)
        acc = r if acc is None else acc + r
        return acc, proj

    xtra = MEM

    def b_body(j, carry):
        x0 = pl.multiple_of(j * 2 * seg, 2 * seg)
        xs = x_ref[pl.ds(x0, 2 * seg), :].astype(f32)
        mem = mem_s[...]
        held = {}

        def tokens_e(g, i, a):
            return jnp.concatenate([a[0:seg], a[seg + xtra:seg + xtra + MEM]], axis=0)

        def olhs_e(g, o):
            held[g] = o[seg - xtra:seg]
            return jnp.concatenate([o[seg:L], o[0:seg - xtra]], axis=0)

        oe, proj_e = step(jnp.concatenate([xs[0:seg + xtra], mem], axis=0), tokens_e, olhs_e)
        mem = oe[0:MEM].astype(bf16).astype(f32)

        def tokens_o(g, i, a):
            return jnp.concatenate([proj_e[g][i][seg:seg + xtra], a], axis=0)

        def olhs_o(g, o):
            return jnp.concatenate([o[seg:L], held[g], o[0:seg]], axis=0)

        oo, _ = step(jnp.concatenate([xs[seg + xtra:2 * seg], mem], axis=0), tokens_o, olhs_o)
        mem_s[...] = oo[0:MEM].astype(bf16).astype(f32)
        b = jnp.concatenate([oe[MEM:], oo[MEM:]], axis=0)
        gate = jax.nn.sigmoid(jnp.sum(xs * gw, axis=-1, keepdims=True))
        o_ref[pl.ds(x0, 2 * seg), :] = (gate * a_s[pl.ds(x0, 2 * seg), :]
                                        + (1.0 - gate) * b).astype(o_ref.dtype)
        return carry

    jax.lax.fori_loop(0, nseg // 2, b_body, 0)


@functools.partial(jax.jit, static_argnames=("B_seg_len",))
def pallas_gated_mix__mha_block__memory_aug_recurrent_mem_tr__prompt_kernel(
    A_x: jax.Array,
    A_wqkv: jax.Array,
    A_wo: jax.Array,
    B_x: jax.Array,
    B_mem0: jax.Array,
    B_Wq: jax.Array,
    B_Wk: jax.Array,
    B_Wv: jax.Array,
    B_Wo: jax.Array,
    B_seg_len: int,
    gate_w: jax.Array,
):
    del B_x
    seg = int(B_seg_len)
    assert A_x.shape == (1, S, D) and B_Wq.shape == (D, HB, DHB) and B_mem0.shape == (1, MEM, D)
    assert S % (2 * seg) == 0 and seg % 16 == 0 and seg > MEM

    scratch = [
        pltpu.VMEM((S, D), bf16),
        pltpu.VMEM((S // 2, D), u32),
        pltpu.VMEM((HA * 16, S), u32),
        pltpu.VMEM((S, GH * TQ), f32),
        pltpu.VMEM((S, GH * TQ), f32),
        pltpu.VMEM((S // 2, GH * TQ), u32),
        pltpu.VMEM((S // 2, GH * TQ), u32),
        pltpu.VMEM((8, GH * TQ), f32),
        pltpu.VMEM((8, GH * TQ), f32),
        pltpu.VMEM((8, GH * TQ), f32),
        pltpu.VMEM((D, S), f32),
        pltpu.VMEM((S, D), f32),
        pltpu.VMEM((D, HB, DHB), bf16),
        pltpu.VMEM((D, HB, DHB), bf16),
        pltpu.VMEM((D, HB, DHB), bf16),
        pltpu.VMEM((HB * DHB, D), bf16),
        pltpu.VMEM((D // 2, HB * DHB), u32),
        pltpu.VMEM((D // 2, HB * DHB), u32),
        pltpu.VMEM((D // 2, HB * DHB), u32),
        pltpu.VMEM((HB * DHB // 2, D), u32),
        pltpu.VMEM((MEM, D), f32),
        pltpu.SemaphoreType.DMA((4,)),
    ]
    vmem_full = pl.BlockSpec(memory_space=pltpu.VMEM)
    hbm_full = pl.BlockSpec(memory_space=pl.ANY)
    out = pl.pallas_call(
        functools.partial(_kernel, seg=seg),
        out_shape=jax.ShapeDtypeStruct((S, D), A_x.dtype),
        in_specs=[vmem_full] * 4 + [hbm_full] * 4 + [vmem_full],
        out_specs=vmem_full,
        scratch_shapes=scratch,
        compiler_params=pltpu.CompilerParams(vmem_limit_bytes=120 * 1024 * 1024),
        name="gated_mix_mha_rmt",
    )(
        A_x.reshape(S, D),
        A_wqkv,
        A_wo,
        B_mem0.reshape(MEM, D),
        B_Wq,
        B_Wk,
        B_Wv,
        B_Wo.reshape(HB * DHB, D),
        gate_w.reshape(1, D),
    )
    return out.reshape(1, S, D)
```

```python
import functools
import math

import jax
import jax.numpy as jnp
import jax.experimental.pallas as pl
import jax.experimental.pallas.tpu as pltpu

f32, bf16, u32 = jnp.float32, jnp.bfloat16, jnp.uint32

S, D = 2048, 512
HA, DHA = 32, 16
TQ = 128
GH = 128 // DHA
NG = HA // GH
CH = 32
CHK = 128
SKEW = (S // CHK) // 2
HB, DHB, MEM = 32, 128, 8
BND = (0, 10, 22, 32)
NGB = len(BND) - 1


def _pack(x):
    return pltpu.bitcast(x, u32)


def _unpack(x):
    return pltpu.bitcast(x, bf16)


def _kernel(x_ref, wqkv_ref, woa_ref, mem0_ref, wq_hbm, wk_hbm, wv_hbm, wob_hbm, gw_ref,
            o_ref,
            q_s, kp, vta, st0, st1, pt0, pt1, m0, m1, mc, ot_s, a_s,
            wq_raw, wk_raw, wv_raw, wo_raw, wq_p, wk_p, wv_p, wo_p, mem_s, sems, *, seg):
    w_copies = [pltpu.make_async_copy(src, dst, sems.at[i]) for i, (src, dst) in enumerate(
        [(wq_hbm, wq_raw), (wk_hbm, wk_raw), (wv_hbm, wv_raw), (wob_hbm, wo_raw)])]
    for cp in w_copies:
        cp.start()

    x = x_ref[...]
    q = jnp.dot(x, wqkv_ref[:, 0:D], preferred_element_type=f32)
    q_s[...] = (q.astype(bf16) * DHA ** -0.5).astype(bf16)
    kp[...] = _pack(jnp.dot(x, wqkv_ref[:, D:2 * D], preferred_element_type=f32).astype(bf16))
    v = jnp.dot(x, wqkv_ref[:, 2 * D:3 * D], preferred_element_type=f32)
    vt = v.T
    rowi = jax.lax.broadcasted_iota(jnp.int32, (16, S), 0)
    ones_blk = jnp.where(rowi == 0, 1.0, 0.0).astype(bf16)
    for h in range(HA):
        vta[pl.ds(h * 16, 8), :] = _pack(vt[h * DHA:(h + 1) * DHA, :].astype(bf16))
        vta[pl.ds(h * 16 + 8, 8), :] = _pack(ones_blk)

    lane_head = jax.lax.broadcasted_iota(jnp.int32, (TQ, 128), 1) // DHA
    NC = S // CHK

    def idx(i):
        g = i % NG
        qb = i // NG
        return g, pl.multiple_of(g * 128, 128), pl.multiple_of(qb * TQ, TQ)

    def build_qm(i):
        g, g0, q0 = idx(i)
        qblk = q_s[pl.ds(q0, TQ), pl.ds(g0, 128)]
        return jnp.concatenate(
            [jnp.where(lane_head == h, qblk, jnp.zeros_like(qblk)) for h in range(GH)], axis=0)

    def scores_chunk(i, qm, st, c, macc):
        g, g0, q0 = idx(i)
        kg = _unpack(kp[c * CHK // 2:(c + 1) * CHK // 2, pl.ds(g0, 128)])
        s = jax.lax.dot_general(kg, qm, (((1,), (1,)), ((), ())), preferred_element_type=f32)
        st[c * CHK:(c + 1) * CHK, :] = s
        cm = jnp.max(s.reshape(CHK // 8, 8, GH * TQ), axis=0)
        return cm if macc is None else jnp.maximum(macc, cm)

    def finish_max(macc, mm):
        mm[...] = jnp.broadcast_to(jnp.max(macc, axis=0, keepdims=True), (8, GH * TQ))

    def softmax_chunk(st, mb, pt, c):
        for cc in range(c * CHK // CH, (c + 1) * CHK // CH):
            p = jnp.exp(st[cc * CH:(cc + 1) * CH, :] - mb)
            pt[cc * CH // 2:(cc + 1) * CH // 2, :] = _pack(p.astype(bf16))

    def pv_chunk(i, pt, c, R):
        g, g0, q0 = idx(i)
        out = []
        for h in range(GH):
            r0 = pl.multiple_of((g * GH + h) * 16, 16)
            lhs = _unpack(vta[pl.ds(r0, 16), c * CHK:(c + 1) * CHK])
            r = jnp.dot(lhs, _unpack(pt[c * CHK // 2:(c + 1) * CHK // 2, h * TQ:(h + 1) * TQ]),
                        preferred_element_type=f32)
            out.append(r if R is None else R[h] + r)
        return out

    def unit(i, st_cur, m_cur, pt, st_oth, m_oth, macc):
        u1 = jnp.minimum(i + 1, NU - 1)
        u2 = jnp.minimum(i + 2, NU - 1)
        qm1 = build_qm(u1)
        qm2 = None
        mb = jnp.concatenate([m_cur[...]] * (CH // 8), axis=0)
        R = None
        for c in range(NC):
            cs = c + SKEW
            if cs < NC:
                macc = scores_chunk(u1, qm1, st_oth, cs, macc)
            else:
                if cs == NC:
                    finish_max(macc, m_oth)
                    macc = None
                    qm2 = build_qm(u2)
                macc = scores_chunk(u2, qm2, st_cur, cs - NC, macc)
            softmax_chunk(st_cur, mb, pt, c)
            R = pv_chunk(i, pt, c, R)
        g, g0, q0 = idx(i)
        for h in range(GH):
            ot_s[pl.ds(pl.multiple_of(g0 + h * DHA, DHA), DHA), pl.ds(q0, TQ)] = (
                R[h][0:DHA] / R[h][DHA:DHA + 1])
        return macc

    NU = NG * (S // TQ)
    qm0 = build_qm(0)
    macc = None
    for c in range(NC):
        macc = scores_chunk(0, qm0, st0, c, macc)
    finish_max(macc, m0)
    qm1 = build_qm(1)
    macc = None
    for c in range(SKEW):
        macc = scores_chunk(1, qm1, st1, c, macc)
    mc[...] = macc

    for cp in w_copies:
        cp.wait()
    NIT = NU // 2
    DR = D // NIT
    OR = HB * DHB // NIT

    def pack_weights(j):
        d0 = pl.multiple_of(j * DR, DR)
        p0 = pl.multiple_of(j * (DR // 2), DR // 2)
        for raw, packed in ((wq_raw, wq_p), (wk_raw, wk_p), (wv_raw, wv_p)):
            packed[pl.ds(p0, DR // 2), :] = _pack(raw[pl.ds(d0, DR)].reshape(DR, HB * DHB))
        o0 = pl.multiple_of(j * OR, OR)
        po0 = pl.multiple_of(j * (OR // 2), OR // 2)
        wo_p[pl.ds(po0, OR // 2), :] = _pack(wo_raw[pl.ds(o0, OR), :])

    def a_body(j, carry):
        i = 2 * j
        macc = unit(i, st0, m0, pt0, st1, m1, mc[...])
        pack_weights(j)
        mc[...] = unit(i + 1, st1, m1, pt1, st0, m0, macc)
        return carry

    jax.lax.fori_loop(0, NIT, a_body, 0)
    a_s[...] = jnp.dot(ot_s[...].T.astype(bf16), woa_ref[...], preferred_element_type=f32)

    mem_s[...] = mem0_ref[...].astype(f32)
    gw = gw_ref[...].astype(f32)

    L = MEM + seg
    nseg = S // seg
    scale = DHB ** -0.5
    row = jax.lax.broadcasted_iota(jnp.int32, (L, L), 0)
    col = jax.lax.broadcasted_iota(jnp.int32, (L, L), 1)
    mask = (row >= seg) | (col >= seg) | (col <= row)

    def proj1(hb, w_p, g):
        return jnp.dot(hb, _unpack(w_p[:, BND[g] * DHB:BND[g + 1] * DHB]), preferred_element_type=f32)

    def scores_b(q, k):
        q = q.astype(bf16)
        k = k.astype(bf16)
        return [jax.lax.dot_general(q[:, hd * DHB:(hd + 1) * DHB], k[:, hd * DHB:(hd + 1) * DHB],
                                    (((1,), (1,)), ((), ())), preferred_element_type=f32)
                for hd in range(q.shape[1] // DHB)]

    def softmax_b(scs):
        out = []
        for sc in scs:
            sc = jnp.where(mask, sc * scale, -1e9)
            mx = jnp.max(sc, axis=-1, keepdims=True)
            p = jnp.exp(sc - mx)
            l = jnp.sum(p, axis=-1, keepdims=True)
            out.append((p / l).astype(bf16))
        return out

    def pv_b(ps, v):
        v = v.astype(bf16)
        return jnp.concatenate(
            [jnp.dot(ps[hd], v[:, hd * DHB:(hd + 1) * DHB], preferred_element_type=f32)
             for hd in range(len(ps))], axis=1)

    def oproj1(lhs, g):
        return jnp.dot(lhs.astype(bf16), _unpack(wo_p[BND[g] * DHB // 2:BND[g + 1] * DHB // 2, :]),
                       preferred_element_type=f32)

    def step(hrows, tokens, olhs):
        hb = hrows.astype(bf16)
        proj = [None] * NGB
        proj[0] = [proj1(hb, w, 0) for w in (wq_p, wk_p, wv_p)]
        acc = None
        o_g = [None] * NGB
        for g in range(NGB):
            q, k, v = (tokens(g, i, a) for i, a in enumerate(proj[g]))
            scs = scores_b(q, k)
            if g + 1 < NGB:
                nq = proj1(hb, wq_p, g + 1)
            if g >= 1:
                r = oproj1(olhs(g - 1, o_g[g - 1]), g - 1)
                acc = r if acc is None else acc + r
            ps = softmax_b(scs)
            o_g[g] = pv_b(ps, v)
            if g + 1 < NGB:
                proj[g + 1] = [nq, proj1(hb, wk_p, g + 1), proj1(hb, wv_p, g + 1)]
        r = oproj1(olhs(NGB - 1, o_g[NGB - 1]), NGB - 1)
        acc = r if acc is None else acc + r
        return acc, proj

    xtra = MEM

    def b_body(j, carry):
        x0 = pl.multiple_of(j * 2 * seg, 2 * seg)
        xs = x_ref[pl.ds(x0, 2 * seg), :].astype(f32)
        mem = mem_s[...]
        held = {}

        def tokens_e(g, i, a):
            return jnp.concatenate([a[0:seg], a[seg + xtra:seg + xtra + MEM]], axis=0)

        def olhs_e(g, o):
            held[g] = o[seg - xtra:seg]
            return jnp.concatenate([o[seg:L], o[0:seg - xtra]], axis=0)

        oe, proj_e = step(jnp.concatenate([xs[0:seg + xtra], mem], axis=0), tokens_e, olhs_e)
        mem = oe[0:MEM].astype(bf16).astype(f32)

        def tokens_o(g, i, a):
            return jnp.concatenate([proj_e[g][i][seg:seg + xtra], a], axis=0)

        def olhs_o(g, o):
            return jnp.concatenate([o[seg:L], held[g], o[0:seg]], axis=0)

        oo, _ = step(jnp.concatenate([xs[seg + xtra:2 * seg], mem], axis=0), tokens_o, olhs_o)
        mem_s[...] = oo[0:MEM].astype(bf16).astype(f32)
        b = jnp.concatenate([oe[MEM:], oo[MEM:]], axis=0)
        gate = jax.nn.sigmoid(jnp.sum(xs * gw, axis=-1, keepdims=True))
        o_ref[pl.ds(x0, 2 * seg), :] = (gate * a_s[pl.ds(x0, 2 * seg), :]
                                        + (1.0 - gate) * b).astype(o_ref.dtype)
        return carry

    jax.lax.fori_loop(0, nseg // 2, b_body, 0)


@functools.partial(jax.jit, static_argnames=("B_seg_len",))
def pallas_gated_mix__mha_block__memory_aug_recurrent_mem_tr__prompt_kernel(
    A_x: jax.Array,
    A_wqkv: jax.Array,
    A_wo: jax.Array,
    B_x: jax.Array,
    B_mem0: jax.Array,
    B_Wq: jax.Array,
    B_Wk: jax.Array,
    B_Wv: jax.Array,
    B_Wo: jax.Array,
    B_seg_len: int,
    gate_w: jax.Array,
):
    del B_x
    seg = int(B_seg_len)
    assert A_x.shape == (1, S, D) and B_Wq.shape == (D, HB, DHB) and B_mem0.shape == (1, MEM, D)
    assert S % (2 * seg) == 0 and seg % 16 == 0 and seg > MEM

    scratch = [
        pltpu.VMEM((S, D), bf16),
        pltpu.VMEM((S // 2, D), u32),
        pltpu.VMEM((HA * 16, S), u32),
        pltpu.VMEM((S, GH * TQ), f32),
        pltpu.VMEM((S, GH * TQ), f32),
        pltpu.VMEM((S // 2, GH * TQ), u32),
        pltpu.VMEM((S // 2, GH * TQ), u32),
        pltpu.VMEM((8, GH * TQ), f32),
        pltpu.VMEM((8, GH * TQ), f32),
        pltpu.VMEM((8, GH * TQ), f32),
        pltpu.VMEM((D, S), f32),
        pltpu.VMEM((S, D), f32),
        pltpu.VMEM((D, HB, DHB), bf16),
        pltpu.VMEM((D, HB, DHB), bf16),
        pltpu.VMEM((D, HB, DHB), bf16),
        pltpu.VMEM((HB * DHB, D), bf16),
        pltpu.VMEM((D // 2, HB * DHB), u32),
        pltpu.VMEM((D // 2, HB * DHB), u32),
        pltpu.VMEM((D // 2, HB * DHB), u32),
        pltpu.VMEM((HB * DHB // 2, D), u32),
        pltpu.VMEM((MEM, D), f32),
        pltpu.SemaphoreType.DMA((4,)),
    ]
    vmem_full = pl.BlockSpec(memory_space=pltpu.VMEM)
    hbm_full = pl.BlockSpec(memory_space=pl.ANY)
    out = pl.pallas_call(
        functools.partial(_kernel, seg=seg),
        out_shape=jax.ShapeDtypeStruct((S, D), A_x.dtype),
        in_specs=[vmem_full] * 4 + [hbm_full] * 4 + [vmem_full],
        out_specs=vmem_full,
        scratch_shapes=scratch,
        compiler_params=pltpu.CompilerParams(vmem_limit_bytes=120 * 1024 * 1024),
        name="gated_mix_mha_rmt",
    )(
        A_x.reshape(S, D),
        A_wqkv,
        A_wo,
        B_mem0.reshape(MEM, D),
        B_Wq,
        B_Wk,
        B_Wv,
        B_Wo.reshape(HB * DHB, D),
        gate_w.reshape(1, D),
    )
    return out.reshape(1, S, D)
```

```python
import functools
import math

import jax
import jax.numpy as jnp
import jax.experimental.pallas as pl
import jax.experimental.pallas.tpu as pltpu

f32, bf16, u32 = jnp.float32, jnp.bfloat16, jnp.uint32

S, D = 2048, 512
HA, DHA = 32, 16
TQ = 128
GH = 128 // DHA
NG = HA // GH
CH = 32
CHK = 128
SKEW = (S // CHK) // 2
HB, DHB, MEM = 32, 128, 8
BND = (0, 10, 22, 32)
NGB = len(BND) - 1


def _pack(x):
    return pltpu.bitcast(x, u32)


def _unpack(x):
    return pltpu.bitcast(x, bf16)


def _kernel(x_ref, wqkv_ref, woa_ref, mem0_ref, wq_hbm, wk_hbm, wv_hbm, wob_hbm, gw_ref,
            o_ref,
            q_s, kp, vta, st0, st1, pt0, pt1, m0, m1, mc, ot_s, a_s,
            wq_raw, wk_raw, wv_raw, wo_raw, wq_p, wk_p, wv_p, wo_p, mem_s, sems, *, seg):
    w_copies = [pltpu.make_async_copy(src, dst, sems.at[i]) for i, (src, dst) in enumerate(
        [(wq_hbm, wq_raw), (wk_hbm, wk_raw), (wv_hbm, wv_raw), (wob_hbm, wo_raw)])]
    for cp in w_copies:
        cp.start()

    x = x_ref[...]
    q = jnp.dot(x, wqkv_ref[:, 0:D], preferred_element_type=f32)
    q_s[...] = (q.astype(bf16) * DHA ** -0.5).astype(bf16)
    kp[...] = _pack(jnp.dot(x, wqkv_ref[:, D:2 * D], preferred_element_type=f32).astype(bf16))
    v = jnp.dot(x, wqkv_ref[:, 2 * D:3 * D], preferred_element_type=f32)
    vt = v.T
    rowi = jax.lax.broadcasted_iota(jnp.int32, (16, S), 0)
    ones_blk = jnp.where(rowi == 0, 1.0, 0.0).astype(bf16)
    for h in range(HA):
        vta[pl.ds(h * 16, 8), :] = _pack(vt[h * DHA:(h + 1) * DHA, :].astype(bf16))
        vta[pl.ds(h * 16 + 8, 8), :] = _pack(ones_blk)

    lane_head = jax.lax.broadcasted_iota(jnp.int32, (TQ, 128), 1) // DHA
    NC = S // CHK

    def idx(i):
        g = i % NG
        qb = i // NG
        return g, pl.multiple_of(g * 128, 128), pl.multiple_of(qb * TQ, TQ)

    def build_qm(i):
        g, g0, q0 = idx(i)
        qblk = q_s[pl.ds(q0, TQ), pl.ds(g0, 128)]
        return jnp.concatenate(
            [jnp.where(lane_head == h, qblk, jnp.zeros_like(qblk)) for h in range(GH)], axis=0)

    def scores_chunk(i, qm, st, c, macc):
        g, g0, q0 = idx(i)
        kg = _unpack(kp[c * CHK // 2:(c + 1) * CHK // 2, pl.ds(g0, 128)])
        s = jax.lax.dot_general(kg, qm, (((1,), (1,)), ((), ())), preferred_element_type=f32)
        st[c * CHK:(c + 1) * CHK, :] = s
        cm = jnp.max(s.reshape(CHK // 8, 8, GH * TQ), axis=0)
        return cm if macc is None else jnp.maximum(macc, cm)

    def finish_max(macc, mm):
        mm[...] = jnp.broadcast_to(jnp.max(macc, axis=0, keepdims=True), (8, GH * TQ))

    def softmax_chunk(st, mb, pt, c):
        for cc in range(c * CHK // CH, (c + 1) * CHK // CH):
            p = jnp.exp(st[cc * CH:(cc + 1) * CH, :] - mb)
            pt[cc * CH // 2:(cc + 1) * CH // 2, :] = _pack(p.astype(bf16))

    def pv_chunk(i, pt, c, R):
        g, g0, q0 = idx(i)
        out = []
        for h in range(GH):
            r0 = pl.multiple_of((g * GH + h) * 16, 16)
            lhs = _unpack(vta[pl.ds(r0, 16), c * CHK:(c + 1) * CHK])
            r = jnp.dot(lhs, _unpack(pt[c * CHK // 2:(c + 1) * CHK // 2, h * TQ:(h + 1) * TQ]),
                        preferred_element_type=f32)
            out.append(r if R is None else R[h] + r)
        return out

    def unit(i, st_cur, m_cur, pt, st_oth, m_oth, macc):
        u1 = jnp.minimum(i + 1, NU - 1)
        u2 = jnp.minimum(i + 2, NU - 1)
        qm1 = build_qm(u1)
        qm2 = None
        mb = jnp.concatenate([m_cur[...]] * (CH // 8), axis=0)
        R = None
        for c in range(NC):
            cs = c + SKEW
            if cs < NC:
                macc = scores_chunk(u1, qm1, st_oth, cs, macc)
            else:
                if cs == NC:
                    finish_max(macc, m_oth)
                    macc = None
                    qm2 = build_qm(u2)
                macc = scores_chunk(u2, qm2, st_cur, cs - NC, macc)
            softmax_chunk(st_cur, mb, pt, c)
            R = pv_chunk(i, pt, c, R)
        g, g0, q0 = idx(i)
        for h in range(GH):
            ot_s[pl.ds(pl.multiple_of(g0 + h * DHA, DHA), DHA), pl.ds(q0, TQ)] = (
                R[h][0:DHA] / R[h][DHA:DHA + 1])
        return macc

    NU = NG * (S // TQ)
    qm0 = build_qm(0)
    macc = None
    for c in range(NC):
        macc = scores_chunk(0, qm0, st0, c, macc)
    finish_max(macc, m0)
    qm1 = build_qm(1)
    macc = None
    for c in range(SKEW):
        macc = scores_chunk(1, qm1, st1, c, macc)
    mc[...] = macc

    def a_body(j, carry):
        i = 2 * j
        macc = unit(i, st0, m0, pt0, st1, m1, mc[...])
        mc[...] = unit(i + 1, st1, m1, pt1, st0, m0, macc)
        return carry

    jax.lax.fori_loop(0, NU // 2, a_body, 0)
    a_s[...] = jnp.dot(ot_s[...].T.astype(bf16), woa_ref[...], preferred_element_type=f32)

    for cp, raw, packed in zip(w_copies[:3], (wq_raw, wk_raw, wv_raw), (wq_p, wk_p, wv_p)):
        cp.wait()
        packed[...] = _pack(raw[...].reshape(D, HB * DHB))
    w_copies[3].wait()
    wo_p[...] = _pack(wo_raw[...])
    pltpu.touch(wq_p); pltpu.touch(wk_p); pltpu.touch(wv_p); pltpu.touch(wo_p)
    for raw, packed in zip((wq_raw, wk_raw, wv_raw), (wq_p, wk_p, wv_p)):
        packed[...] = _pack(raw[...].reshape(D, HB * DHB))
    wo_p[...] = _pack(wo_raw[...])
    mem_s[...] = mem0_ref[...].astype(f32)
    gw = gw_ref[...].astype(f32)

    L = MEM + seg
    nseg = S // seg
    scale = DHB ** -0.5
    row = jax.lax.broadcasted_iota(jnp.int32, (L, L), 0)
    col = jax.lax.broadcasted_iota(jnp.int32, (L, L), 1)
    mask = (row >= seg) | (col >= seg) | (col <= row)

    def proj1(hb, w_p, g):
        return jnp.dot(hb, _unpack(w_p[:, BND[g] * DHB:BND[g + 1] * DHB]), preferred_element_type=f32)

    def scores_b(q, k):
        q = q.astype(bf16)
        k = k.astype(bf16)
        return [jax.lax.dot_general(q[:, hd * DHB:(hd + 1) * DHB], k[:, hd * DHB:(hd + 1) * DHB],
                                    (((1,), (1,)), ((), ())), preferred_element_type=f32)
                for hd in range(q.shape[1] // DHB)]

    def softmax_b(scs):
        out = []
        for sc in scs:
            sc = jnp.where(mask, sc * scale, -1e9)
            mx = jnp.max(sc, axis=-1, keepdims=True)
            p = jnp.exp(sc - mx)
            l = jnp.sum(p, axis=-1, keepdims=True)
            out.append((p / l).astype(bf16))
        return out

    def pv_b(ps, v):
        v = v.astype(bf16)
        return jnp.concatenate(
            [jnp.dot(ps[hd], v[:, hd * DHB:(hd + 1) * DHB], preferred_element_type=f32)
             for hd in range(len(ps))], axis=1)

    def oproj1(lhs, g):
        return jnp.dot(lhs.astype(bf16), _unpack(wo_p[BND[g] * DHB // 2:BND[g + 1] * DHB // 2, :]),
                       preferred_element_type=f32)

    def step(hrows, tokens, olhs):
        hb = hrows.astype(bf16)
        proj = [None] * NGB
        proj[0] = [proj1(hb, w, 0) for w in (wq_p, wk_p, wv_p)]
        acc = None
        o_g = [None] * NGB
        for g in range(NGB):
            q, k, v = (tokens(g, i, a) for i, a in enumerate(proj[g]))
            scs = scores_b(q, k)
            if g + 1 < NGB:
                nq = proj1(hb, wq_p, g + 1)
            if g >= 1:
                r = oproj1(olhs(g - 1, o_g[g - 1]), g - 1)
                acc = r if acc is None else acc + r
            ps = softmax_b(scs)
            o_g[g] = pv_b(ps, v)
            if g + 1 < NGB:
                proj[g + 1] = [nq, proj1(hb, wk_p, g + 1), proj1(hb, wv_p, g + 1)]
        r = oproj1(olhs(NGB - 1, o_g[NGB - 1]), NGB - 1)
        acc = r if acc is None else acc + r
        return acc, proj

    xtra = MEM

    def b_body(j, carry):
        x0 = pl.multiple_of(j * 2 * seg, 2 * seg)
        xs = x_ref[pl.ds(x0, 2 * seg), :].astype(f32)
        mem = mem_s[...]
        held = {}

        def tokens_e(g, i, a):
            return jnp.concatenate([a[0:seg], a[seg + xtra:seg + xtra + MEM]], axis=0)

        def olhs_e(g, o):
            held[g] = o[seg - xtra:seg]
            return jnp.concatenate([o[seg:L], o[0:seg - xtra]], axis=0)

        oe, proj_e = step(jnp.concatenate([xs[0:seg + xtra], mem], axis=0), tokens_e, olhs_e)
        mem = oe[0:MEM].astype(bf16).astype(f32)

        def tokens_o(g, i, a):
            return jnp.concatenate([proj_e[g][i][seg:seg + xtra], a], axis=0)

        def olhs_o(g, o):
            return jnp.concatenate([o[seg:L], held[g], o[0:seg]], axis=0)

        oo, _ = step(jnp.concatenate([xs[seg + xtra:2 * seg], mem], axis=0), tokens_o, olhs_o)
        mem_s[...] = oo[0:MEM].astype(bf16).astype(f32)
        b = jnp.concatenate([oe[MEM:], oo[MEM:]], axis=0)
        gate = jax.nn.sigmoid(jnp.sum(xs * gw, axis=-1, keepdims=True))
        o_ref[pl.ds(x0, 2 * seg), :] = (gate * a_s[pl.ds(x0, 2 * seg), :]
                                        + (1.0 - gate) * b).astype(o_ref.dtype)
        return carry

    jax.lax.fori_loop(0, nseg // 2, b_body, 0)


@functools.partial(jax.jit, static_argnames=("B_seg_len",))
def pallas_gated_mix__mha_block__memory_aug_recurrent_mem_tr__prompt_kernel(
    A_x: jax.Array,
    A_wqkv: jax.Array,
    A_wo: jax.Array,
    B_x: jax.Array,
    B_mem0: jax.Array,
    B_Wq: jax.Array,
    B_Wk: jax.Array,
    B_Wv: jax.Array,
    B_Wo: jax.Array,
    B_seg_len: int,
    gate_w: jax.Array,
):
    del B_x
    seg = int(B_seg_len)
    assert A_x.shape == (1, S, D) and B_Wq.shape == (D, HB, DHB) and B_mem0.shape == (1, MEM, D)
    assert S % (2 * seg) == 0 and seg % 16 == 0 and seg > MEM

    scratch = [
        pltpu.VMEM((S, D), bf16),
        pltpu.VMEM((S // 2, D), u32),
        pltpu.VMEM((HA * 16, S), u32),
        pltpu.VMEM((S, GH * TQ), f32),
        pltpu.VMEM((S, GH * TQ), f32),
        pltpu.VMEM((S // 2, GH * TQ), u32),
        pltpu.VMEM((S // 2, GH * TQ), u32),
        pltpu.VMEM((8, GH * TQ), f32),
        pltpu.VMEM((8, GH * TQ), f32),
        pltpu.VMEM((8, GH * TQ), f32),
        pltpu.VMEM((D, S), f32),
        pltpu.VMEM((S, D), f32),
        pltpu.VMEM((D, HB, DHB), bf16),
        pltpu.VMEM((D, HB, DHB), bf16),
        pltpu.VMEM((D, HB, DHB), bf16),
        pltpu.VMEM((HB * DHB, D), bf16),
        pltpu.VMEM((D // 2, HB * DHB), u32),
        pltpu.VMEM((D // 2, HB * DHB), u32),
        pltpu.VMEM((D // 2, HB * DHB), u32),
        pltpu.VMEM((HB * DHB // 2, D), u32),
        pltpu.VMEM((MEM, D), f32),
        pltpu.SemaphoreType.DMA((4,)),
    ]
    vmem_full = pl.BlockSpec(memory_space=pltpu.VMEM)
    hbm_full = pl.BlockSpec(memory_space=pl.ANY)
    out = pl.pallas_call(
        functools.partial(_kernel, seg=seg),
        out_shape=jax.ShapeDtypeStruct((S, D), A_x.dtype),
        in_specs=[vmem_full] * 4 + [hbm_full] * 4 + [vmem_full],
        out_specs=vmem_full,
        scratch_shapes=scratch,
        compiler_params=pltpu.CompilerParams(vmem_limit_bytes=120 * 1024 * 1024),
        name="gated_mix_mha_rmt",
    )(
        A_x.reshape(S, D),
        A_wqkv,
        A_wo,
        B_mem0.reshape(MEM, D),
        B_Wq,
        B_Wk,
        B_Wv,
        B_Wo.reshape(HB * DHB, D),
        gate_w.reshape(1, D),
    )
    return out.reshape(1, S, D)
```

```python
import functools
import math

import jax
import jax.numpy as jnp
import jax.experimental.pallas as pl
import jax.experimental.pallas.tpu as pltpu

f32, bf16, u32 = jnp.float32, jnp.bfloat16, jnp.uint32

S, D = 2048, 512
HA, DHA = 32, 16
TQ = 128
GH = 128 // DHA
NG = HA // GH
CH = 32
CHK = 128
SKEW = (S // CHK) // 2
HB, DHB, MEM = 32, 128, 8
BND = (0, 10, 22, 32)
NGB = len(BND) - 1


def _pack(x):
    return pltpu.bitcast(x, u32)


def _unpack(x):
    return pltpu.bitcast(x, bf16)


def _kernel(x_ref, wqkv_ref, woa_ref, mem0_ref, wq_hbm, wk_hbm, wv_hbm, wob_hbm, gw_ref,
            o_ref,
            q_s, kp, vta, st0, st1, pt0, pt1, m0, m1, mc, ot_s, a_s,
            wq_raw, wk_raw, wv_raw, wo_raw, wq_p, wk_p, wv_p, wo_p, mem_s, sems, *, seg):
    w_copies = [pltpu.make_async_copy(src, dst, sems.at[i]) for i, (src, dst) in enumerate(
        [(wq_hbm, wq_raw), (wk_hbm, wk_raw), (wv_hbm, wv_raw), (wob_hbm, wo_raw)])]
    for cp in w_copies:
        cp.start()

    x = x_ref[...]
    q = jnp.dot(x, wqkv_ref[:, 0:D], preferred_element_type=f32)
    q_s[...] = (q.astype(bf16) * DHA ** -0.5).astype(bf16)
    kp[...] = _pack(jnp.dot(x, wqkv_ref[:, D:2 * D], preferred_element_type=f32).astype(bf16))
    v = jnp.dot(x, wqkv_ref[:, 2 * D:3 * D], preferred_element_type=f32)
    vt = v.T
    rowi = jax.lax.broadcasted_iota(jnp.int32, (16, S), 0)
    ones_blk = jnp.where(rowi == 0, 1.0, 0.0).astype(bf16)
    for h in range(HA):
        vta[pl.ds(h * 16, 8), :] = _pack(vt[h * DHA:(h + 1) * DHA, :].astype(bf16))
        vta[pl.ds(h * 16 + 8, 8), :] = _pack(ones_blk)

    lane_head = jax.lax.broadcasted_iota(jnp.int32, (TQ, 128), 1) // DHA
    NC = S // CHK

    def idx(i):
        g = i % NG
        qb = i // NG
        return g, pl.multiple_of(g * 128, 128), pl.multiple_of(qb * TQ, TQ)

    def build_qm(i):
        g, g0, q0 = idx(i)
        qblk = q_s[pl.ds(q0, TQ), pl.ds(g0, 128)]
        return jnp.concatenate(
            [jnp.where(lane_head == h, qblk, jnp.zeros_like(qblk)) for h in range(GH)], axis=0)

    def scores_chunk(i, qm, st, c, macc):
        g, g0, q0 = idx(i)
        kg = _unpack(kp[c * CHK // 2:(c + 1) * CHK // 2, pl.ds(g0, 128)])
        s = jax.lax.dot_general(kg, qm, (((1,), (1,)), ((), ())), preferred_element_type=f32)
        st[c * CHK:(c + 1) * CHK, :] = s
        cm = jnp.max(s.reshape(CHK // 8, 8, GH * TQ), axis=0)
        return cm if macc is None else jnp.maximum(macc, cm)

    def finish_max(macc, mm):
        mm[...] = jnp.broadcast_to(jnp.max(macc, axis=0, keepdims=True), (8, GH * TQ))

    def softmax_chunk(st, mb, pt, c):
        for cc in range(c * CHK // CH, (c + 1) * CHK // CH):
            p = jnp.exp(st[cc * CH:(cc + 1) * CH, :] - mb)
            pt[cc * CH // 2:(cc + 1) * CH // 2, :] = _pack(p.astype(bf16))

    def pv_chunk(i, pt, c, R):
        g, g0, q0 = idx(i)
        out = []
        for h in range(GH):
            r0 = pl.multiple_of((g * GH + h) * 16, 16)
            lhs = _unpack(vta[pl.ds(r0, 16), c * CHK:(c + 1) * CHK])
            r = jnp.dot(lhs, _unpack(pt[c * CHK // 2:(c + 1) * CHK // 2, h * TQ:(h + 1) * TQ]),
                        preferred_element_type=f32)
            out.append(r if R is None else R[h] + r)
        return out

    def unit(i, st_cur, m_cur, pt, st_oth, m_oth, macc, side):
        u1 = jnp.minimum(i + 1, NU - 1)
        u2 = jnp.minimum(i + 2, NU - 1)
        qm1 = build_qm(u1)
        qm2 = None
        mb = jnp.concatenate([m_cur[...]] * (CH // 8), axis=0)
        R = None
        for c in range(NC):
            cs = c + SKEW
            if cs < NC:
                macc = scores_chunk(u1, qm1, st_oth, cs, macc)
            else:
                if cs == NC:
                    finish_max(macc, m_oth)
                    macc = None
                    qm2 = build_qm(u2)
                macc = scores_chunk(u2, qm2, st_cur, cs - NC, macc)
            if c % SIDE_EVERY == 1:
                side[c // SIDE_EVERY]()
            softmax_chunk(st_cur, mb, pt, c)
            R = pv_chunk(i, pt, c, R)
        g, g0, q0 = idx(i)
        for h in range(GH):
            ot_s[pl.ds(pl.multiple_of(g0 + h * DHA, DHA), DHA), pl.ds(q0, TQ)] = (
                R[h][0:DHA] / R[h][DHA:DHA + 1])
        return macc

    NU = NG * (S // TQ)
    qm0 = build_qm(0)
    macc = None
    for c in range(NC):
        macc = scores_chunk(0, qm0, st0, c, macc)
    finish_max(macc, m0)
    qm1 = build_qm(1)
    macc = None
    for c in range(SKEW):
        macc = scores_chunk(1, qm1, st1, c, macc)
    mc[...] = macc

    for cp in w_copies:
        cp.wait()
    NIT = NU // 2
    DR = D // NIT
    OR = HB * DHB // NIT

    SIDE_EVERY = NC // 4

    def pack_qkv_piece(raw, packed, j, half):
        def run():
            d0 = pl.multiple_of(j * DR, DR)
            p0 = pl.multiple_of(j * (DR // 2), DR // 2)
            hh = HB // 2
            packed[pl.ds(p0, DR // 2), half * hh * DHB:(half + 1) * hh * DHB] = _pack(
                raw[pl.ds(d0, DR), half * hh:(half + 1) * hh, :].reshape(DR, hh * DHB))
        return run

    def pack_wo_piece(j, half):
        def run():
            o0 = pl.multiple_of(j * OR + half * (OR // 2), OR // 2)
            po0 = pl.multiple_of(j * (OR // 2) + half * (OR // 4), OR // 4)
            wo_p[pl.ds(po0, OR // 4), :] = _pack(wo_raw[pl.ds(o0, OR // 2), :])
        return run

    def a_body(j, carry):
        i = 2 * j
        side0 = [pack_qkv_piece(wq_raw, wq_p, j, 0), pack_qkv_piece(wq_raw, wq_p, j, 1),
                 pack_qkv_piece(wk_raw, wk_p, j, 0), pack_qkv_piece(wk_raw, wk_p, j, 1)]
        side1 = [pack_qkv_piece(wv_raw, wv_p, j, 0), pack_qkv_piece(wv_raw, wv_p, j, 1),
                 pack_wo_piece(j, 0), pack_wo_piece(j, 1)]
        macc = unit(i, st0, m0, pt0, st1, m1, mc[...], side0)
        mc[...] = unit(i + 1, st1, m1, pt1, st0, m0, macc, side1)
        return carry

    jax.lax.fori_loop(0, NIT, a_body, 0)
    a_s[...] = jnp.dot(ot_s[...].T.astype(bf16), woa_ref[...], preferred_element_type=f32)

    mem_s[...] = mem0_ref[...].astype(f32)
    gw = gw_ref[...].astype(f32)

    L = MEM + seg
    nseg = S // seg
    scale = DHB ** -0.5
    row = jax.lax.broadcasted_iota(jnp.int32, (L, L), 0)
    col = jax.lax.broadcasted_iota(jnp.int32, (L, L), 1)
    mask = (row >= seg) | (col >= seg) | (col <= row)

    def proj1(hb, w_p, g):
        return jnp.dot(hb, _unpack(w_p[:, BND[g] * DHB:BND[g + 1] * DHB]), preferred_element_type=f32)

    def scores_b(q, k):
        q = q.astype(bf16)
        k = k.astype(bf16)
        return [jax.lax.dot_general(q[:, hd * DHB:(hd + 1) * DHB], k[:, hd * DHB:(hd + 1) * DHB],
                                    (((1,), (1,)), ((), ())), preferred_element_type=f32)
                for hd in range(q.shape[1] // DHB)]

    def softmax_b(scs):
        out = []
        for sc in scs:
            sc = jnp.where(mask, sc * scale, -1e9)
            mx = jnp.max(sc, axis=-1, keepdims=True)
            p = jnp.exp(sc - mx)
            l = jnp.sum(p, axis=-1, keepdims=True)
            out.append((p / l).astype(bf16))
        return out

    def pv_b(ps, v):
        v = v.astype(bf16)
        return jnp.concatenate(
            [jnp.dot(ps[hd], v[:, hd * DHB:(hd + 1) * DHB], preferred_element_type=f32)
             for hd in range(len(ps))], axis=1)

    def oproj1(lhs, g):
        return jnp.dot(lhs.astype(bf16), _unpack(wo_p[BND[g] * DHB // 2:BND[g + 1] * DHB // 2, :]),
                       preferred_element_type=f32)

    def step(hrows, tokens, olhs):
        hb = hrows.astype(bf16)
        proj = [None] * NGB
        proj[0] = [proj1(hb, w, 0) for w in (wq_p, wk_p, wv_p)]
        acc = None
        o_g = [None] * NGB
        for g in range(NGB):
            q, k, v = (tokens(g, i, a) for i, a in enumerate(proj[g]))
            scs = scores_b(q, k)
            if g + 1 < NGB:
                nq = proj1(hb, wq_p, g + 1)
            if g >= 1:
                r = oproj1(olhs(g - 1, o_g[g - 1]), g - 1)
                acc = r if acc is None else acc + r
            ps = softmax_b(scs)
            o_g[g] = pv_b(ps, v)
            if g + 1 < NGB:
                proj[g + 1] = [nq, proj1(hb, wk_p, g + 1), proj1(hb, wv_p, g + 1)]
        r = oproj1(olhs(NGB - 1, o_g[NGB - 1]), NGB - 1)
        acc = r if acc is None else acc + r
        return acc, proj

    xtra = MEM

    def b_body(j, carry):
        x0 = pl.multiple_of(j * 2 * seg, 2 * seg)
        xs = x_ref[pl.ds(x0, 2 * seg), :].astype(f32)
        mem = mem_s[...]
        held = {}

        def tokens_e(g, i, a):
            return jnp.concatenate([a[0:seg], a[seg + xtra:seg + xtra + MEM]], axis=0)

        def olhs_e(g, o):
            held[g] = o[seg - xtra:seg]
            return jnp.concatenate([o[seg:L], o[0:seg - xtra]], axis=0)

        oe, proj_e = step(jnp.concatenate([xs[0:seg + xtra], mem], axis=0), tokens_e, olhs_e)
        mem = oe[0:MEM].astype(bf16).astype(f32)

        def tokens_o(g, i, a):
            return jnp.concatenate([proj_e[g][i][seg:seg + xtra], a], axis=0)

        def olhs_o(g, o):
            return jnp.concatenate([o[seg:L], held[g], o[0:seg]], axis=0)

        oo, _ = step(jnp.concatenate([xs[seg + xtra:2 * seg], mem], axis=0), tokens_o, olhs_o)
        mem_s[...] = oo[0:MEM].astype(bf16).astype(f32)
        b = jnp.concatenate([oe[MEM:], oo[MEM:]], axis=0)
        gate = jax.nn.sigmoid(jnp.sum(xs * gw, axis=-1, keepdims=True))
        o_ref[pl.ds(x0, 2 * seg), :] = (gate * a_s[pl.ds(x0, 2 * seg), :]
                                        + (1.0 - gate) * b).astype(o_ref.dtype)
        return carry

    jax.lax.fori_loop(0, nseg // 2, b_body, 0)


@functools.partial(jax.jit, static_argnames=("B_seg_len",))
def pallas_gated_mix__mha_block__memory_aug_recurrent_mem_tr__prompt_kernel(
    A_x: jax.Array,
    A_wqkv: jax.Array,
    A_wo: jax.Array,
    B_x: jax.Array,
    B_mem0: jax.Array,
    B_Wq: jax.Array,
    B_Wk: jax.Array,
    B_Wv: jax.Array,
    B_Wo: jax.Array,
    B_seg_len: int,
    gate_w: jax.Array,
):
    del B_x
    seg = int(B_seg_len)
    assert A_x.shape == (1, S, D) and B_Wq.shape == (D, HB, DHB) and B_mem0.shape == (1, MEM, D)
    assert S % (2 * seg) == 0 and seg % 16 == 0 and seg > MEM

    scratch = [
        pltpu.VMEM((S, D), bf16),
        pltpu.VMEM((S // 2, D), u32),
        pltpu.VMEM((HA * 16, S), u32),
        pltpu.VMEM((S, GH * TQ), f32),
        pltpu.VMEM((S, GH * TQ), f32),
        pltpu.VMEM((S // 2, GH * TQ), u32),
        pltpu.VMEM((S // 2, GH * TQ), u32),
        pltpu.VMEM((8, GH * TQ), f32),
        pltpu.VMEM((8, GH * TQ), f32),
        pltpu.VMEM((8, GH * TQ), f32),
        pltpu.VMEM((D, S), f32),
        pltpu.VMEM((S, D), f32),
        pltpu.VMEM((D, HB, DHB), bf16),
        pltpu.VMEM((D, HB, DHB), bf16),
        pltpu.VMEM((D, HB, DHB), bf16),
        pltpu.VMEM((HB * DHB, D), bf16),
        pltpu.VMEM((D // 2, HB * DHB), u32),
        pltpu.VMEM((D // 2, HB * DHB), u32),
        pltpu.VMEM((D // 2, HB * DHB), u32),
        pltpu.VMEM((HB * DHB // 2, D), u32),
        pltpu.VMEM((MEM, D), f32),
        pltpu.SemaphoreType.DMA((4,)),
    ]
    vmem_full = pl.BlockSpec(memory_space=pltpu.VMEM)
    hbm_full = pl.BlockSpec(memory_space=pl.ANY)
    out = pl.pallas_call(
        functools.partial(_kernel, seg=seg),
        out_shape=jax.ShapeDtypeStruct((S, D), A_x.dtype),
        in_specs=[vmem_full] * 4 + [hbm_full] * 4 + [vmem_full],
        out_specs=vmem_full,
        scratch_shapes=scratch,
        compiler_params=pltpu.CompilerParams(vmem_limit_bytes=120 * 1024 * 1024),
        name="gated_mix_mha_rmt",
    )(
        A_x.reshape(S, D),
        A_wqkv,
        A_wo,
        B_mem0.reshape(MEM, D),
        B_Wq,
        B_Wk,
        B_Wv,
        B_Wo.reshape(HB * DHB, D),
        gate_w.reshape(1, D),
    )
    return out.reshape(1, S, D)
```

```python
import functools
import math

import jax
import jax.numpy as jnp
import jax.experimental.pallas as pl
import jax.experimental.pallas.tpu as pltpu

f32, bf16, u32 = jnp.float32, jnp.bfloat16, jnp.uint32

S, D = 2048, 512
HA, DHA = 32, 16
TQ = 128
GH = 128 // DHA
NG = HA // GH
CH = 32
CHK = 128
SKEW = (S // CHK) // 2
HB, DHB, MEM = 32, 128, 8
BND = (0, 10, 22, 32)
NGB = len(BND) - 1


def _pack(x):
    return pltpu.bitcast(x, u32)


def _unpack(x):
    return pltpu.bitcast(x, bf16)


def _kernel(x_ref, wqkv_ref, woa_ref, mem0_ref, wq_hbm, wk_hbm, wv_hbm, wob_hbm, gw_ref,
            o_ref,
            q_s, kp, vta, st0, st1, pt0, pt1, m0, m1, mc, ot_s, a_s,
            wq_raw, wk_raw, wv_raw, wo_raw, wq_p, wk_p, wv_p, wo_p, mem_s, sems, *, seg):
    w_copies = [pltpu.make_async_copy(src, dst, sems.at[i]) for i, (src, dst) in enumerate(
        [(wq_hbm, wq_raw), (wk_hbm, wk_raw), (wv_hbm, wv_raw), (wob_hbm, wo_raw)])]
    for cp in w_copies:
        cp.start()

    x = x_ref[...]
    q = jnp.dot(x, wqkv_ref[:, 0:D], preferred_element_type=f32)
    q_s[...] = (q.astype(bf16) * DHA ** -0.5).astype(bf16)
    kp[...] = _pack(jnp.dot(x, wqkv_ref[:, D:2 * D], preferred_element_type=f32).astype(bf16))
    v = jnp.dot(x, wqkv_ref[:, 2 * D:3 * D], preferred_element_type=f32)
    vt = v.T
    rowi = jax.lax.broadcasted_iota(jnp.int32, (16, S), 0)
    ones_blk = jnp.where(rowi == 0, 1.0, 0.0).astype(bf16)
    for h in range(HA):
        vta[pl.ds(h * 16, 8), :] = _pack(vt[h * DHA:(h + 1) * DHA, :].astype(bf16))
        vta[pl.ds(h * 16 + 8, 8), :] = _pack(ones_blk)

    lane_head = jax.lax.broadcasted_iota(jnp.int32, (TQ, 128), 1) // DHA
    NC = S // CHK

    def idx(i):
        g = i % NG
        qb = i // NG
        return g, pl.multiple_of(g * 128, 128), pl.multiple_of(qb * TQ, TQ)

    def build_qm(i):
        g, g0, q0 = idx(i)
        qblk = q_s[pl.ds(q0, TQ), pl.ds(g0, 128)]
        return jnp.concatenate(
            [jnp.where(lane_head == h, qblk, jnp.zeros_like(qblk)) for h in range(GH)], axis=0)

    def scores_chunk(i, qm, st, c, macc):
        g, g0, q0 = idx(i)
        kg = _unpack(kp[c * CHK // 2:(c + 1) * CHK // 2, pl.ds(g0, 128)])
        s = jax.lax.dot_general(kg, qm, (((1,), (1,)), ((), ())), preferred_element_type=f32)
        st[c * CHK:(c + 1) * CHK, :] = s
        cm = jnp.max(s.reshape(CHK // 8, 8, GH * TQ), axis=0)
        return cm if macc is None else jnp.maximum(macc, cm)

    def finish_max(macc, mm):
        mm[...] = jnp.broadcast_to(jnp.max(macc, axis=0, keepdims=True), (8, GH * TQ))

    def softmax_chunk(st, mb, pt, c):
        for cc in range(c * CHK // CH, (c + 1) * CHK // CH):
            p = jnp.exp(st[cc * CH:(cc + 1) * CH, :] - mb)
            pt[cc * CH // 2:(cc + 1) * CH // 2, :] = _pack(p.astype(bf16))

    def pv_chunk(i, pt, c, R):
        g, g0, q0 = idx(i)
        out = []
        for h in range(GH):
            r0 = pl.multiple_of((g * GH + h) * 16, 16)
            lhs = _unpack(vta[pl.ds(r0, 16), c * CHK:(c + 1) * CHK])
            r = jnp.dot(lhs, _unpack(pt[c * CHK // 2:(c + 1) * CHK // 2, h * TQ:(h + 1) * TQ]),
                        preferred_element_type=f32)
            out.append(r if R is None else R[h] + r)
        return out

    def unit(i, st_cur, m_cur, pt, st_oth, m_oth, macc, has_u1=True, has_u2=True):
        qm1 = build_qm(i + 1) if has_u1 else None
        qm2 = None
        mb = jnp.concatenate([m_cur[...]] * (CH // 8), axis=0)
        R = None
        for c in range(NC):
            cs = c + SKEW
            if cs < NC:
                if has_u1:
                    macc = scores_chunk(i + 1, qm1, st_oth, cs, macc)
            else:
                if cs == NC:
                    if has_u1:
                        finish_max(macc, m_oth)
                    macc = None
                    if has_u2:
                        qm2 = build_qm(i + 2)
                if has_u2:
                    macc = scores_chunk(i + 2, qm2, st_cur, cs - NC, macc)
            softmax_chunk(st_cur, mb, pt, c)
            R = pv_chunk(i, pt, c, R)
        g, g0, q0 = idx(i)
        for h in range(GH):
            ot_s[pl.ds(pl.multiple_of(g0 + h * DHA, DHA), DHA), pl.ds(q0, TQ)] = (
                R[h][0:DHA] / R[h][DHA:DHA + 1])
        return macc

    NU = NG * (S // TQ)
    qm0 = build_qm(0)
    macc = None
    for c in range(NC):
        macc = scores_chunk(0, qm0, st0, c, macc)
    finish_max(macc, m0)
    qm1 = build_qm(1)
    macc = None
    for c in range(SKEW):
        macc = scores_chunk(1, qm1, st1, c, macc)
    mc[...] = macc

    def a_body(j, carry):
        i = 2 * j
        macc = unit(i, st0, m0, pt0, st1, m1, mc[...])
        mc[...] = unit(i + 1, st1, m1, pt1, st0, m0, macc)
        return carry

    jax.lax.fori_loop(0, NU // 2 - 1, a_body, 0)
    macc = unit(NU - 2, st0, m0, pt0, st1, m1, mc[...], has_u2=False)
    unit(NU - 1, st1, m1, pt1, st0, m0, macc, has_u1=False, has_u2=False)
    a_s[...] = jnp.dot(ot_s[...].T.astype(bf16), woa_ref[...], preferred_element_type=f32)

    for cp, raw, packed in zip(w_copies[:3], (wq_raw, wk_raw, wv_raw), (wq_p, wk_p, wv_p)):
        cp.wait()
        packed[...] = _pack(raw[...].reshape(D, HB * DHB))
    w_copies[3].wait()
    wo_p[...] = _pack(wo_raw[...])
    mem_s[...] = mem0_ref[...].astype(f32)
    gw = gw_ref[...].astype(f32)

    L = MEM + seg
    nseg = S // seg
    scale = DHB ** -0.5
    row = jax.lax.broadcasted_iota(jnp.int32, (L, L), 0)
    col = jax.lax.broadcasted_iota(jnp.int32, (L, L), 1)
    mask = (row >= seg) | (col >= seg) | (col <= row)

    def proj1(hb, w_p, g):
        return jnp.dot(hb, _unpack(w_p[:, BND[g] * DHB:BND[g + 1] * DHB]), preferred_element_type=f32)

    def scores_b(q, k):
        q = q.astype(bf16)
        k = k.astype(bf16)
        return [jax.lax.dot_general(q[:, hd * DHB:(hd + 1) * DHB], k[:, hd * DHB:(hd + 1) * DHB],
                                    (((1,), (1,)), ((), ())), preferred_element_type=f32)
                for hd in range(q.shape[1] // DHB)]

    def softmax_b(scs):
        out = []
        for sc in scs:
            sc = jnp.where(mask, sc * scale, -1e9)
            mx = jnp.max(sc, axis=-1, keepdims=True)
            p = jnp.exp(sc - mx)
            l = jnp.sum(p, axis=-1, keepdims=True)
            out.append((p / l).astype(bf16))
        return out

    def pv_b(ps, v):
        v = v.astype(bf16)
        return jnp.concatenate(
            [jnp.dot(ps[hd], v[:, hd * DHB:(hd + 1) * DHB], preferred_element_type=f32)
             for hd in range(len(ps))], axis=1)

    def oproj1(lhs, g):
        return jnp.dot(lhs.astype(bf16), _unpack(wo_p[BND[g] * DHB // 2:BND[g + 1] * DHB // 2, :]),
                       preferred_element_type=f32)

    def step(hrows, tokens, olhs):
        hb = hrows.astype(bf16)
        proj = [None] * NGB
        proj[0] = [proj1(hb, w, 0) for w in (wq_p, wk_p, wv_p)]
        acc = None
        o_g = [None] * NGB
        for g in range(NGB):
            q, k, v = (tokens(g, i, a) for i, a in enumerate(proj[g]))
            scs = scores_b(q, k)
            if g + 1 < NGB:
                nq = proj1(hb, wq_p, g + 1)
            if g >= 1:
                r = oproj1(olhs(g - 1, o_g[g - 1]), g - 1)
                acc = r if acc is None else acc + r
            ps = softmax_b(scs)
            o_g[g] = pv_b(ps, v)
            if g + 1 < NGB:
                proj[g + 1] = [nq, proj1(hb, wk_p, g + 1), proj1(hb, wv_p, g + 1)]
        r = oproj1(olhs(NGB - 1, o_g[NGB - 1]), NGB - 1)
        acc = r if acc is None else acc + r
        return acc, proj

    xtra = MEM

    def b_body(j, carry):
        x0 = pl.multiple_of(j * 2 * seg, 2 * seg)
        xs = x_ref[pl.ds(x0, 2 * seg), :].astype(f32)
        mem = mem_s[...]
        held = {}

        def tokens_e(g, i, a):
            return jnp.concatenate([a[0:seg], a[seg + xtra:seg + xtra + MEM]], axis=0)

        def olhs_e(g, o):
            held[g] = o[seg - xtra:seg]
            return jnp.concatenate([o[seg:L], o[0:seg - xtra]], axis=0)

        oe, proj_e = step(jnp.concatenate([xs[0:seg + xtra], mem], axis=0), tokens_e, olhs_e)
        mem = oe[0:MEM].astype(bf16).astype(f32)

        def tokens_o(g, i, a):
            return jnp.concatenate([proj_e[g][i][seg:seg + xtra], a], axis=0)

        def olhs_o(g, o):
            return jnp.concatenate([o[seg:L], held[g], o[0:seg]], axis=0)

        oo, _ = step(jnp.concatenate([xs[seg + xtra:2 * seg], mem], axis=0), tokens_o, olhs_o)
        mem_s[...] = oo[0:MEM].astype(bf16).astype(f32)
        b = jnp.concatenate([oe[MEM:], oo[MEM:]], axis=0)
        gate = jax.nn.sigmoid(jnp.sum(xs * gw, axis=-1, keepdims=True))
        o_ref[pl.ds(x0, 2 * seg), :] = (gate * a_s[pl.ds(x0, 2 * seg), :]
                                        + (1.0 - gate) * b).astype(o_ref.dtype)
        return carry

    jax.lax.fori_loop(0, nseg // 2, b_body, 0)


@functools.partial(jax.jit, static_argnames=("B_seg_len",))
def pallas_gated_mix__mha_block__memory_aug_recurrent_mem_tr__prompt_kernel(
    A_x: jax.Array,
    A_wqkv: jax.Array,
    A_wo: jax.Array,
    B_x: jax.Array,
    B_mem0: jax.Array,
    B_Wq: jax.Array,
    B_Wk: jax.Array,
    B_Wv: jax.Array,
    B_Wo: jax.Array,
    B_seg_len: int,
    gate_w: jax.Array,
):
    del B_x
    seg = int(B_seg_len)
    assert A_x.shape == (1, S, D) and B_Wq.shape == (D, HB, DHB) and B_mem0.shape == (1, MEM, D)
    assert S % (2 * seg) == 0 and seg % 16 == 0 and seg > MEM

    scratch = [
        pltpu.VMEM((S, D), bf16),
        pltpu.VMEM((S // 2, D), u32),
        pltpu.VMEM((HA * 16, S), u32),
        pltpu.VMEM((S, GH * TQ), f32),
        pltpu.VMEM((S, GH * TQ), f32),
        pltpu.VMEM((S // 2, GH * TQ), u32),
        pltpu.VMEM((S // 2, GH * TQ), u32),
        pltpu.VMEM((8, GH * TQ), f32),
        pltpu.VMEM((8, GH * TQ), f32),
        pltpu.VMEM((8, GH * TQ), f32),
        pltpu.VMEM((D, S), f32),
        pltpu.VMEM((S, D), f32),
        pltpu.VMEM((D, HB, DHB), bf16),
        pltpu.VMEM((D, HB, DHB), bf16),
        pltpu.VMEM((D, HB, DHB), bf16),
        pltpu.VMEM((HB * DHB, D), bf16),
        pltpu.VMEM((D // 2, HB * DHB), u32),
        pltpu.VMEM((D // 2, HB * DHB), u32),
        pltpu.VMEM((D // 2, HB * DHB), u32),
        pltpu.VMEM((HB * DHB // 2, D), u32),
        pltpu.VMEM((MEM, D), f32),
        pltpu.SemaphoreType.DMA((4,)),
    ]
    vmem_full = pl.BlockSpec(memory_space=pltpu.VMEM)
    hbm_full = pl.BlockSpec(memory_space=pl.ANY)
    out = pl.pallas_call(
        functools.partial(_kernel, seg=seg),
        out_shape=jax.ShapeDtypeStruct((S, D), A_x.dtype),
        in_specs=[vmem_full] * 4 + [hbm_full] * 4 + [vmem_full],
        out_specs=vmem_full,
        scratch_shapes=scratch,
        compiler_params=pltpu.CompilerParams(vmem_limit_bytes=120 * 1024 * 1024),
        name="gated_mix_mha_rmt",
    )(
        A_x.reshape(S, D),
        A_wqkv,
        A_wo,
        B_mem0.reshape(MEM, D),
        B_Wq,
        B_Wk,
        B_Wv,
        B_Wo.reshape(HB * DHB, D),
        gate_w.reshape(1, D),
    )
    return out.reshape(1, S, D)
```

```python
import functools

import jax
import jax.numpy as jnp
import jax.experimental.pallas as pl
import jax.experimental.pallas.tpu as pltpu

f32, bf16, u32 = jnp.float32, jnp.bfloat16, jnp.uint32

S, D = 2048, 512
HA, DHA = 32, 16
TQ = 128
GH = 128 // DHA
NG = HA // GH
CH = 32
CHK = 128
SKEW = 4
HB, DHB, MEM = 32, 128, 8
BND = (0, 10, 22, 32)
NGB = len(BND) - 1


def _pack(x):
    return pltpu.bitcast(x, u32)


def _unpack(x):
    return pltpu.bitcast(x, bf16)


def _kernel(x_ref, wqkv_ref, woa_ref, mem0_ref, wq_hbm, wk_hbm, wv_hbm, wob_hbm, gw_ref,
            o_ref,
            q_s, kp, vta, st0, st1, pt0, pt1, m0, m1, mc, ot_s, a_s,
            wq_raw, wk_raw, wv_raw, wo_raw, wq_p, wk_p, wv_p, wo_p, mem_s, sems, *, seg):
    w_copies = [pltpu.make_async_copy(src, dst, sems.at[i]) for i, (src, dst) in enumerate(
        [(wq_hbm, wq_raw), (wk_hbm, wk_raw), (wv_hbm, wv_raw), (wob_hbm, wo_raw)])]
    for cp in w_copies:
        cp.start()

    x = x_ref[...]
    q = jnp.dot(x, wqkv_ref[:, 0:D], preferred_element_type=f32)
    q_s[...] = (q.astype(bf16) * DHA ** -0.5).astype(bf16)
    kp[...] = _pack(jnp.dot(x, wqkv_ref[:, D:2 * D], preferred_element_type=f32).astype(bf16))
    v = jnp.dot(x, wqkv_ref[:, 2 * D:3 * D], preferred_element_type=f32)
    vt = v.T
    rowi = jax.lax.broadcasted_iota(jnp.int32, (16, S), 0)
    ones_blk = jnp.where(rowi == 0, 1.0, 0.0).astype(bf16)
    for h in range(HA):
        vta[pl.ds(h * 16, 8), :] = _pack(vt[h * DHA:(h + 1) * DHA, :].astype(bf16))
        vta[pl.ds(h * 16 + 8, 8), :] = _pack(ones_blk)

    lane_head = jax.lax.broadcasted_iota(jnp.int32, (TQ, 128), 1) // DHA
    NC = S // CHK

    def idx(i):
        g = i % NG
        qb = i // NG
        return g, pl.multiple_of(g * 128, 128), pl.multiple_of(qb * TQ, TQ)

    def build_qm(i):
        g, g0, q0 = idx(i)
        qblk = q_s[pl.ds(q0, TQ), pl.ds(g0, 128)]
        return jnp.concatenate(
            [jnp.where(lane_head == h, qblk, jnp.zeros_like(qblk)) for h in range(GH)], axis=0)

    def scores_chunk(i, qm, st, c, macc):
        g, g0, q0 = idx(i)
        kg = _unpack(kp[c * CHK // 2:(c + 1) * CHK // 2, pl.ds(g0, 128)])
        s = jax.lax.dot_general(kg, qm, (((1,), (1,)), ((), ())), preferred_element_type=f32)
        st[c * CHK:(c + 1) * CHK, :] = s
        cm = jnp.max(s.reshape(CHK // 8, 8, GH * TQ), axis=0)
        return cm if macc is None else jnp.maximum(macc, cm)

    def finish_max(macc, mm):
        mm[...] = jnp.broadcast_to(jnp.max(macc, axis=0, keepdims=True), (8, GH * TQ))

    def softmax_chunk(st, mb, pt, c):
        for cc in range(c * CHK // CH, (c + 1) * CHK // CH):
            p = jnp.exp(st[cc * CH:(cc + 1) * CH, :] - mb)
            pt[cc * CH // 2:(cc + 1) * CH // 2, :] = _pack(p.astype(bf16))

    def pv_chunk(i, pt, c, R):
        g, g0, q0 = idx(i)
        out = []
        for h in range(GH):
            r0 = pl.multiple_of((g * GH + h) * 16, 16)
            lhs = _unpack(vta[pl.ds(r0, 16), c * CHK:(c + 1) * CHK])
            r = jnp.dot(lhs, _unpack(pt[c * CHK // 2:(c + 1) * CHK // 2, h * TQ:(h + 1) * TQ]),
                        preferred_element_type=f32)
            out.append(r if R is None else R[h] + r)
        return out

    def unit(i, st_cur, m_cur, pt, st_oth, m_oth, macc):
        u1 = jnp.minimum(i + 1, NU - 1)
        u2 = jnp.minimum(i + 2, NU - 1)
        qm1 = build_qm(u1)
        qm2 = None
        mb = jnp.concatenate([m_cur[...]] * (CH // 8), axis=0)
        R = None
        for c in range(NC):
            cs = c + SKEW
            if cs < NC:
                macc = scores_chunk(u1, qm1, st_oth, cs, macc)
            else:
                if cs == NC:
                    finish_max(macc, m_oth)
                    macc = None
                    qm2 = build_qm(u2)
                macc = scores_chunk(u2, qm2, st_cur, cs - NC, macc)
            softmax_chunk(st_cur, mb, pt, c)
            R = pv_chunk(i, pt, c, R)
        g, g0, q0 = idx(i)
        for h in range(GH):
            ot_s[pl.ds(pl.multiple_of(g0 + h * DHA, DHA), DHA), pl.ds(q0, TQ)] = (
                R[h][0:DHA] / R[h][DHA:DHA + 1])
        return macc

    NU = NG * (S // TQ)
    qm0 = build_qm(0)
    macc = None
    for c in range(NC):
        macc = scores_chunk(0, qm0, st0, c, macc)
    finish_max(macc, m0)
    qm1 = build_qm(1)
    macc = None
    for c in range(SKEW):
        macc = scores_chunk(1, qm1, st1, c, macc)
    mc[...] = macc

    def a_body(j, carry):
        i = 2 * j
        macc = unit(i, st0, m0, pt0, st1, m1, mc[...])
        mc[...] = unit(i + 1, st1, m1, pt1, st0, m0, macc)
        return carry

    jax.lax.fori_loop(0, NU // 2, a_body, 0)
    a_s[...] = jnp.dot(ot_s[...].T.astype(bf16), woa_ref[...], preferred_element_type=f32)

    for cp, raw, packed in zip(w_copies[:3], (wq_raw, wk_raw, wv_raw), (wq_p, wk_p, wv_p)):
        cp.wait()
        packed[...] = _pack(raw[...].reshape(D, HB * DHB))
    w_copies[3].wait()
    wo_p[...] = _pack(wo_raw[...])
    mem_s[...] = mem0_ref[...].astype(f32)
    gw = gw_ref[...].astype(f32)

    L = MEM + seg
    nseg = S // seg
    scale = DHB ** -0.5
    row = jax.lax.broadcasted_iota(jnp.int32, (L, L), 0)
    col = jax.lax.broadcasted_iota(jnp.int32, (L, L), 1)
    mask = (row >= seg) | (col >= seg) | (col <= row)

    def proj1(hb, w_p, g):
        return jnp.dot(hb, _unpack(w_p[:, BND[g] * DHB:BND[g + 1] * DHB]), preferred_element_type=f32)

    def scores_b(q, k):
        q = q.astype(bf16)
        k = k.astype(bf16)
        return [jax.lax.dot_general(q[:, hd * DHB:(hd + 1) * DHB], k[:, hd * DHB:(hd + 1) * DHB],
                                    (((1,), (1,)), ((), ())), preferred_element_type=f32)
                for hd in range(q.shape[1] // DHB)]

    def softmax_b(scs):
        out = []
        for sc in scs:
            sc = jnp.where(mask, sc * scale, -1e9)
            mx = jnp.max(sc, axis=-1, keepdims=True)
            p = jnp.exp(sc - mx)
            l = jnp.sum(p, axis=-1, keepdims=True)
            out.append((p / l).astype(bf16))
        return out

    def pv_b(ps, v):
        v = v.astype(bf16)
        return jnp.concatenate(
            [jnp.dot(ps[hd], v[:, hd * DHB:(hd + 1) * DHB], preferred_element_type=f32)
             for hd in range(len(ps))], axis=1)

    def oproj1(lhs, g):
        return jnp.dot(lhs.astype(bf16), _unpack(wo_p[BND[g] * DHB // 2:BND[g + 1] * DHB // 2, :]),
                       preferred_element_type=f32)

    def step(hrows, tokens, olhs):
        hb = hrows.astype(bf16)
        proj = [None] * NGB
        proj[0] = [proj1(hb, w, 0) for w in (wq_p, wk_p, wv_p)]
        acc = None
        o_g = [None] * NGB
        for g in range(NGB):
            q, k, v = (tokens(g, i, a) for i, a in enumerate(proj[g]))
            scs = scores_b(q, k)
            if g + 1 < NGB:
                nq = proj1(hb, wq_p, g + 1)
            if g >= 1:
                r = oproj1(olhs(g - 1, o_g[g - 1]), g - 1)
                acc = r if acc is None else acc + r
            ps = softmax_b(scs)
            o_g[g] = pv_b(ps, v)
            if g + 1 < NGB:
                proj[g + 1] = [nq, proj1(hb, wk_p, g + 1), proj1(hb, wv_p, g + 1)]
        r = oproj1(olhs(NGB - 1, o_g[NGB - 1]), NGB - 1)
        acc = r if acc is None else acc + r
        return acc, proj

    xtra = MEM

    def b_body(j, carry):
        x0 = pl.multiple_of(j * 2 * seg, 2 * seg)
        xs = x_ref[pl.ds(x0, 2 * seg), :].astype(f32)
        mem = mem_s[...]
        held = {}

        def tokens_e(g, i, a):
            return jnp.concatenate([a[0:seg], a[seg + xtra:seg + xtra + MEM]], axis=0)

        def olhs_e(g, o):
            held[g] = o[seg - xtra:seg]
            return jnp.concatenate([o[seg:L], o[0:seg - xtra]], axis=0)

        oe, proj_e = step(jnp.concatenate([xs[0:seg + xtra], mem], axis=0), tokens_e, olhs_e)
        mem = oe[0:MEM].astype(bf16).astype(f32)

        def tokens_o(g, i, a):
            return jnp.concatenate([proj_e[g][i][seg:seg + xtra], a], axis=0)

        def olhs_o(g, o):
            return jnp.concatenate([o[seg:L], held[g], o[0:seg]], axis=0)

        oo, _ = step(jnp.concatenate([xs[seg + xtra:2 * seg], mem], axis=0), tokens_o, olhs_o)
        mem_s[...] = oo[0:MEM].astype(bf16).astype(f32)
        b = jnp.concatenate([oe[MEM:], oo[MEM:]], axis=0)
        gate = jax.nn.sigmoid(jnp.sum(xs * gw, axis=-1, keepdims=True))
        o_ref[pl.ds(x0, 2 * seg), :] = (gate * a_s[pl.ds(x0, 2 * seg), :]
                                        + (1.0 - gate) * b).astype(o_ref.dtype)
        return carry

    jax.lax.fori_loop(0, nseg // 2, b_body, 0)


@functools.partial(jax.jit, static_argnames=("B_seg_len",))
def pallas_gated_mix__mha_block__memory_aug_recurrent_mem_tr__prompt_kernel(
    A_x: jax.Array,
    A_wqkv: jax.Array,
    A_wo: jax.Array,
    B_x: jax.Array,
    B_mem0: jax.Array,
    B_Wq: jax.Array,
    B_Wk: jax.Array,
    B_Wv: jax.Array,
    B_Wo: jax.Array,
    B_seg_len: int,
    gate_w: jax.Array,
):
    del B_x
    seg = int(B_seg_len)
    assert A_x.shape == (1, S, D) and B_Wq.shape == (D, HB, DHB) and B_mem0.shape == (1, MEM, D)
    assert S % (2 * seg) == 0 and seg % 16 == 0 and seg > MEM

    scratch = [
        pltpu.VMEM((S, D), bf16),
        pltpu.VMEM((S // 2, D), u32),
        pltpu.VMEM((HA * 16, S), u32),
        pltpu.VMEM((S, GH * TQ), f32),
        pltpu.VMEM((S, GH * TQ), f32),
        pltpu.VMEM((S // 2, GH * TQ), u32),
        pltpu.VMEM((S // 2, GH * TQ), u32),
        pltpu.VMEM((8, GH * TQ), f32),
        pltpu.VMEM((8, GH * TQ), f32),
        pltpu.VMEM((8, GH * TQ), f32),
        pltpu.VMEM((D, S), f32),
        pltpu.VMEM((S, D), f32),
        pltpu.VMEM((D, HB, DHB), bf16),
        pltpu.VMEM((D, HB, DHB), bf16),
        pltpu.VMEM((D, HB, DHB), bf16),
        pltpu.VMEM((HB * DHB, D), bf16),
        pltpu.VMEM((D // 2, HB * DHB), u32),
        pltpu.VMEM((D // 2, HB * DHB), u32),
        pltpu.VMEM((D // 2, HB * DHB), u32),
        pltpu.VMEM((HB * DHB // 2, D), u32),
        pltpu.VMEM((MEM, D), f32),
        pltpu.SemaphoreType.DMA((4,)),
    ]
    vmem_full = pl.BlockSpec(memory_space=pltpu.VMEM)
    hbm_full = pl.BlockSpec(memory_space=pl.ANY)
    out = pl.pallas_call(
        functools.partial(_kernel, seg=seg),
        out_shape=jax.ShapeDtypeStruct((S, D), A_x.dtype),
        in_specs=[vmem_full] * 4 + [hbm_full] * 4 + [vmem_full],
        out_specs=vmem_full,
        scratch_shapes=scratch,
        compiler_params=pltpu.CompilerParams(vmem_limit_bytes=120 * 1024 * 1024),
        name="gated_mix_mha_rmt",
    )(
        A_x.reshape(S, D),
        A_wqkv,
        A_wo,
        B_mem0.reshape(MEM, D),
        B_Wq,
        B_Wk,
        B_Wv,
        B_Wo.reshape(HB * DHB, D),
        gate_w.reshape(1, D),
    )
    return out.reshape(1, S, D)
```
